```python
import os as _os
_os.environ.setdefault("JAX_PLATFORMS", "cpu")
import jax
import jax.numpy as jnp

def _softmax(x, axis=-1):
    return jax.nn.softmax(x, axis=axis)
def _gelu(x):
    return jax.nn.gelu(x, approximate=True)
def _silu(x):
    return jax.nn.silu(x)
def _sigmoid(x):
    return jax.nn.sigmoid(x)
def _layernorm(x, axis=-1, eps=1e-5):
    m = jnp.mean(x, axis=axis, keepdims=True)
    v = jnp.var(x, axis=axis, keepdims=True)
    return (x - m) / jnp.sqrt(v + eps)
def _scatter_add(tgt, idx, src, axis=0):
    return tgt.at[idx].add(src)
def _segment_sum(src, seg, n):
    return jax.ops.segment_sum(src, seg, n)
class _Rng:
    def __init__(self, key):
        self._k = key
    def _next(self):
        self._k, sub = jax.random.split(self._k)
        return sub
    def normal(self, shape):
        return jax.random.normal(self._next(), shape, dtype=jnp.bfloat16)
    def randint(self, lo, hi, shape):
        return jax.random.randint(self._next(), shape, lo, hi, dtype=jnp.int32)
    def uniform(self, shape, lo=0.0, hi=1.0):
        return jax.random.uniform(self._next(), shape, jnp.bfloat16, lo, hi)
    def permutation(self, n):
        return jax.random.permutation(self._next(), n)


kernel_name = 'sequential_preLN__mha_block__moe_arch_mod__prompt'

def setup_inputs():
    _rng = _Rng(jax.random.key(int.from_bytes(__import__("os").urandom(4), "little")))
    _w = (lambda a: (lambda t: t.astype(jnp.bfloat16) if jnp.issubdtype(t.dtype, jnp.floating) else t)(jnp.asarray(a)))
    def _A_setup():
        B, S, D, H = 1, 2048, 512, 32
        return {
            "x": _w((lambda *s: _rng.normal(s) * 0.05)(B, S, D)),
            "wqkv": _w((lambda *s: _rng.normal(s) * 0.05)(D, 3 * D)),
            "wo": _w((lambda *s: _rng.normal(s) * 0.05)(D, D)),
        }
    _A_in = _A_setup()

    def _B_setup():
        B, S, D, F, C = 1, 2048, 512, 1792, 2
        return {
            "x": _w((lambda *s: _rng.normal(s) * 0.05)(B, S, D)),
            "w_r": _w((lambda *s: _rng.normal(s) * 0.05)(D)),
            "w_gate": _w((lambda *s: _rng.normal(s) * 0.05)(D, F)),
            "w_up": _w((lambda *s: _rng.normal(s) * 0.05)(D, F)),
            "w_down": _w((lambda *s: _rng.normal(s) * 0.05)(F, D)),
        }
    _B_in = _B_setup()

    return {
        "A_x": _A_in["x"],
        "A_wqkv": _A_in["wqkv"],
        "A_wo": _A_in["wo"],
        "B_x": _B_in["x"],
        "B_w_r": _B_in["w_r"],
        "B_w_gate": _B_in["w_gate"],
        "B_w_up": _B_in["w_up"],
        "B_w_down": _B_in["w_down"],
    }

def reference(A_x, A_wqkv, A_wo, B_x, B_w_r, B_w_gate, B_w_up, B_w_down):
    def _A_ref(x, wqkv, wo):
        B, S, D = x.shape
        H = 32
        Dh = D // H
        qkv = (lambda x, *d: x.transpose(*d))((x @ wqkv).reshape(B, S, 3, H, Dh), 2, 0, 3, 1, 4)
        q, k, v = qkv[0], qkv[1], qkv[2]
        scores = jnp.einsum("bhqd,bhkd->bhqk", q, k) * (Dh ** -0.5)
        p = _softmax(scores, axis=-1)
        o = jnp.einsum("bhqk,bhkd->bhqd", p, v)
        return (lambda x, *d: x.transpose(*d))(o, 0, 2, 1, 3).reshape(B, S, D) @ wo

    def _B_ref(x, w_r, w_gate, w_up, w_down):
        B, S, D = x.shape
        C = 2
        r = x @ w_r
        idx = jnp.argsort(-r, axis=-1)[:, :C]
        idx_e = jnp.repeat(idx.reshape(B, C, 1), D, axis=2)
        x_sel = jnp.take_along_axis(x, idx_e, axis=1)
        g = _silu(x_sel @ w_gate)
        u = x_sel @ w_up
        y = (g * u) @ w_down
        r_sel = _sigmoid(jnp.take_along_axis(r, idx, axis=1))
        y = y * r_sel.reshape(B, C, 1)
        b_off = (jnp.arange(B) * S).reshape(B, 1)
        flat_idx = (idx + b_off).reshape(B * C)
        zero = (x * 0.0).reshape(B * S, D)
        upd = _scatter_add(zero, flat_idx, y.reshape(B * C, D), axis=0)
        return x + upd.reshape(B, S, D)

    x = A_x
    h = x + _A_ref(_layernorm(x, axis=-1), A_wqkv, A_wo)
    h2 = h + _B_ref(_layernorm(h, axis=-1), B_w_r, B_w_gate, B_w_up, B_w_down)
    return h2
```

```python
import functools
import math

import jax
import jax.numpy as jnp
from jax import lax
from jax.experimental import pallas as pl
from jax.experimental.pallas import tpu as pltpu

F32 = jnp.float32
BF16 = jnp.bfloat16
U32 = jnp.uint32

S = 2048
D = 512
H = 32
DH = 16
FF = 1792
TQ = 512
CK = 128
NQ = S // TQ
NC = S // CK
NL = TQ // 128
NG = D // 128
OFF = 16
MR = CK - OFF
LAG = 2
NPB = LAG + 2
EPS = 1e-5
QSCALE = (DH ** -0.5) * math.log2(math.e)
NEG = -3.0e38
SAFE_SCORE = 96.0
SAFE_V = 65536.0
VDEP, NPH, PSH = 2, 4, 2


def _pk(x):
    return pltpu.bitcast(x, U32)


def _upk(x):
    return pltpu.bitcast(x, BF16)


def _layernorm(x):
    m = jnp.mean(x, axis=-1, keepdims=True)
    xc = x - m
    v = jnp.mean(xc * xc, axis=-1, keepdims=True)
    return xc * lax.rsqrt(v + EPS)


def _absmax8(x):
    r, c = x.shape
    a = jnp.abs(x).reshape(r // 8, 8, c).max(axis=0)
    out = a[:, 0:128]
    for t in range(1, c // 128):
        out = jnp.maximum(out, a[:, t * 128:(t + 1) * 128])
    return out


def _kernel(x_hbm, wqkv_hbm, wo_hbm, wr_ref, wg_hbm, wu_hbm, wd_hbm, out_hbm,
            x_ref, wq_ref, wk_ref, wv_ref, xb_ref, xi_ref, wo_ref, wg_ref, wu_ref, wd_ref,
            wqt_ref, wvt_ref, k_ref, kf_ref, qt_ref, qf_ref, vt_ref, ot_ref,
            acc_ref, hn_ref, z_ref, y_ref, r_ref,
            p0, p1, p2, p3, sem_x, sem_w, sem_o):
    p_refs = (p0, p1, p2, p3)

    def x_copy(c):
        return pltpu.make_async_copy(x_hbm.at[pl.ds(c * TQ, TQ)], x_ref.at[pl.ds(c * TQ, TQ)], sem_x.at[c])

    def w_copy(i):
        src, dst = ((wqkv_hbm.at[:, pl.ds(D, D)], wk_ref), (wqkv_hbm.at[:, pl.ds(0, D)], wq_ref),
                    (wqkv_hbm.at[:, pl.ds(2 * D, D)], wv_ref), (wo_hbm, wo_ref), (wg_hbm, wg_ref),
                    (wu_hbm, wu_ref), (wd_hbm, wd_ref))[i]
        return pltpu.make_async_copy(src, dst, sem_w.at[i])

    def o_copy(c):
        return pltpu.make_async_copy(y_ref.at[pl.ds(c * TQ, TQ)], out_hbm.at[pl.ds(c * TQ, TQ)], sem_o.at[c])

    x_copy(0).start()
    w_copy(0).start()
    x_copy(1).start()
    w_copy(1).start()
    w_copy(2).start()
    x_copy(2).start()
    x_copy(3).start()

    nt = (((1,), (1,)), ((), ()))
    mx = {}

    def upd(name, v):
        mx[name] = jnp.maximum(mx[name], v) if name in mx else v

    def ln1(c):
        xn = _layernorm(x_ref[c * TQ:(c + 1) * TQ, :].astype(F32))
        xb_ref[c * TQ // 2:(c + 1) * TQ // 2, :] = _pk(xn.astype(BF16))
        x4 = xn.reshape(TQ // 16, 2, 8, D)
        xi_ref[c * TQ // 2:(c + 1) * TQ // 2, :] = pltpu.pack_elementwise(
            [x4[:, 0], x4[:, 1]], packed_dtype=BF16).reshape(TQ // 2, D)

    def kproj(c):
        xb = _upk(xb_ref[c * TQ // 2:(c + 1) * TQ // 2, :])
        kb = jnp.dot(xb, wk_ref[...], preferred_element_type=F32).astype(BF16)
        kf = kb.astype(F32)
        ku = _pk(kb)
        for g in range(NG):
            k_ref[g, c * TQ // 2:(c + 1) * TQ // 2, :] = ku[:, g * 128:(g + 1) * 128]
            for cc in range(TQ // CK):
                row = (c * (TQ // CK) + cc) * OFF
                kf_ref[g, row:row + OFF, :] = kf[cc * CK + MR:(cc + 1) * CK, g * 128:(g + 1) * 128]
        upd('k', _absmax8(kf))

    def qproj(c):
        xb = _upk(xb_ref[c * TQ // 2:(c + 1) * TQ // 2, :])
        qb = (lax.dot_general(wqt_ref[...], xb, nt, preferred_element_type=F32) * QSCALE).astype(BF16)
        qf = qb.astype(F32)
        qu = _pk(qb)
        for g in range(NG):
            qt_ref[g * NQ + c] = qu[g * 64:(g + 1) * 64, :]
            qf_ref[g * NQ + c] = qf[g * 128:(g + 1) * 128, :]
        qa = jnp.abs(qf).reshape(H, 2, 8, TQ)
        upd('q', _absmax8(jnp.sum(qa[:, 0] + qa[:, 1], axis=1)))

    def vproj(c):
        xi = _upk(xi_ref[c * TQ // 2:(c + 1) * TQ // 2, :])
        vb = lax.dot_general(wvt_ref[...], xi, nt, preferred_element_type=F32).astype(BF16)
        vu = _pk(vb)
        for g in range(NG):
            vt_ref[g, :, c * TQ:(c + 1) * TQ] = vu[g * 64:(g + 1) * 64, :]
        upd('v', _absmax8(vb.astype(F32)))

    x_copy(0).wait()
    ln1(0)
    w_copy(0).wait()
    x_copy(1).wait()
    kproj(0)
    ln1(1)
    w_copy(1).wait()
    w_copy(2).wait()
    x_copy(2).wait()
    x_copy(3).wait()
    for i in range(3, 7):
        w_copy(i).start()
    kproj(1)
    wqt_ref[...] = wq_ref[...].astype(F32).T.astype(BF16)
    wvt_ref[...] = wv_ref[...].astype(F32).T.astype(BF16)
    qproj(0)
    ln1(2)
    vproj(0)
    ln1(3)
    for c in range(1, NQ):
        qproj(c)
        vproj(c)
        if c + 1 < NQ:
            kproj(c + 1)
    qmax, kmax, vmax = mx['q'], mx['k'], mx['v']

    bound = jnp.max(qmax) * jnp.max(kmax)
    safe = jnp.logical_and(bound <= SAFE_SCORE, jnp.max(vmax) <= SAFE_V)

    def fast_body(i, carry):
        g = i // NQ
        z0 = i >> 8
        z1 = i >> 9
        st = {}
        deps = [None] * (VDEP * NPH)

        def qk(j, c, slot, n):
            l = st['l'] if c else None

            def emit(r, a, b, l):
                pa = jnp.exp2(a)
                pb = jnp.exp2(b)
                p_refs[slot][z0, r * 8:(r + 1) * 8, :] = pltpu.pack_elementwise([pa, pb], packed_dtype=BF16)
                t = pa + pb
                return t if l is None else l + t

            accs = [[None] * NL for _ in range(OFF // 8)]
            kfs0 = [kf_ref[g, c * OFF + r * 8:c * OFF + (r + 1) * 8, :] for r in range(OFF // 8)]
            kfs = kfs0
            for d in range(DH):
                if d % (DH // NPH) == 0:
                    dep = deps[n * NPH + d // (DH // NPH) + PSH]
                    if dep is not None:
                        dm = jnp.minimum(dep, NEG)
                        kfs = [jnp.maximum(kf, dm) for kf in kfs0]
                kbs = [jnp.broadcast_to(kf[:, j * DH + d:j * DH + d + 1], (8, 128)) for kf in kfs]
                for t in range(NL):
                    qv = jnp.broadcast_to(qf_ref[i, j * DH + d:j * DH + d + 1, t * 128:(t + 1) * 128], (8, 128))
                    for r in range(OFF // 8):
                        x = kbs[r] * qv
                        accs[r][t] = x if accs[r][t] is None else accs[r][t] + x
            rows = [jnp.concatenate(a, axis=1) for a in accs]
            l = emit(MR // 16, rows[0], rows[1], l)

            z = jnp.zeros((8, TQ), U32)
            qm = jnp.concatenate([z] * j + [qt_ref[i, j * 8:(j + 1) * 8, :]] + [z] * (7 - j), axis=0)
            kc = _upk(k_ref[g, c * CK // 2:c * CK // 2 + MR // 2, :])
            s = jnp.dot(kc, _upk(qm), preferred_element_type=F32)
            for ph in range(NPH):
                rr = (ph * (MR // 8) // NPH) * 8
                deps.append(s[rr:rr + 8, 0:128])
            for r in range(MR // 16):
                l = emit(r, s[r * 16:r * 16 + 8], s[r * 16 + 8:r * 16 + 16], l)
            st['l'] = l
            if c == NC - 1:
                st['inv', j] = 1.0 / jnp.sum(l, axis=0, keepdims=True)

        def pv(j, c, slot):
            a = jnp.dot(_upk(vt_ref[g, j * 8:(j + 1) * 8, c * CK:(c + 1) * CK]), _upk(p_refs[slot][z1]),
                        preferred_element_type=F32)
            acc = a if c == 0 else acc_ref[z1] + a
            if c < NC - 1:
                acc_ref[z0] = acc
            else:
                ot_ref[i, j * DH:(j + 1) * DH, :] = (acc * st['inv', j]).astype(BF16)

        pend = []
        n = 0
        for j in range(8):
            for c in range(NC):
                slot = n % NPB
                qk(j, c, slot, n)
                n += 1
                pend.append((j, c, slot))
                if len(pend) > LAG:
                    pv(*pend.pop(0))
        for item in pend:
            pv(*item)
        return carry

    def slow_body(t, carry):
        i = t // 8
        j = t % 8
        g = i // NQ
        rows = lax.broadcasted_iota(jnp.int32, (64, TQ), 0)
        qm = _upk(jnp.where(rows // 8 == j, qt_ref[i], jnp.zeros((64, TQ), U32)))

        def scores(c):
            kc = _upk(k_ref[g, pl.ds(pl.multiple_of(c * (CK // 2), CK // 2), CK // 2), :])
            return jnp.dot(kc, qm, preferred_element_type=F32)

        def max_body(c, m):
            return jnp.maximum(m, jnp.max(scores(c), axis=0, keepdims=True))

        m = lax.fori_loop(0, NC, max_body, jnp.full((1, TQ), -jnp.inf, F32))
        vrow = pl.multiple_of(j * 8, 8)

        def acc_body(c, carry):
            acc, l = carry
            p = jnp.exp2(scores(c) - m)
            p4 = p.reshape(CK // 16, 2, 8, TQ)
            pp = _upk(pltpu.pack_elementwise([p4[:, 0], p4[:, 1]], packed_dtype=BF16).reshape(CK // 2, TQ))
            vc = _upk(vt_ref[g, pl.ds(vrow, 8), pl.ds(pl.multiple_of(c * CK, CK), CK)])
            return (acc + jnp.dot(vc, pp, preferred_element_type=F32),
                    l + jnp.sum(p, axis=0, keepdims=True))

        acc, l = lax.fori_loop(0, NC, acc_body, (jnp.zeros((DH, TQ), F32), jnp.zeros((1, TQ), F32)))
        ot_ref[i, pl.ds(pl.multiple_of(j * DH, DH), DH), :] = (acc / l).astype(BF16)
        return carry

    @pl.when(safe)
    def _():
        lax.fori_loop(0, NG * NQ, fast_body, 0)

    @pl.when(jnp.logical_not(safe))
    def _():
        lax.fori_loop(0, NG * NQ * 8, slow_body, 0)

    w_copy(3).wait()
    tn = (((0,), (0,)), ((), ()))
    wr8 = jnp.broadcast_to(wr_ref[...], (16, D))

    def oproj(c):
        ot = jnp.concatenate([ot_ref[g * NQ + c] for g in range(NG)], axis=0)
        a = lax.dot_general(ot, wo_ref[...], tn, preferred_element_type=F32)
        z_ref[c * TQ:(c + 1) * TQ, :] = x_ref[c * TQ:(c + 1) * TQ, :].astype(F32) + a

    def ln2(c):
        h = z_ref[c * TQ:(c + 1) * TQ, :]
        hn = _layernorm(h)
        zz = h + hn
        hn_ref[c * TQ:(c + 1) * TQ, :] = hn
        z_ref[c * TQ:(c + 1) * TQ, :] = zz
        y_ref[c * TQ:(c + 1) * TQ, :] = zz.astype(BF16)
        r = lax.dot_general(wr8, hn.astype(BF16), nt, preferred_element_type=F32)
        r_ref[:, c * TQ:(c + 1) * TQ] = r[0:8].astype(BF16).astype(F32)

    oproj(0)
    for c in range(NQ):
        if c + 1 < NQ:
            oproj(c + 1)
        ln2(c)
        o_copy(c).start()

    r = r_ref[0:1, :]
    idx = lax.broadcasted_iota(jnp.int32, (1, S), 1)
    m1 = jnp.max(r)
    i1 = jnp.min(jnp.where(r == m1, idx, S))
    r2 = jnp.where(idx == i1, -jnp.inf, r)
    m2 = jnp.max(r2)
    i2 = jnp.min(jnp.where(jnp.logical_and(r2 == m2, idx != i1), idx, S))
    i1 = jnp.clip(i1, 0, S - 1)
    i2 = jnp.clip(i2, 0, S - 1)
    rowi = lax.broadcasted_iota(jnp.int32, (16, D), 0)
    xs = jnp.where(rowi == 0, jnp.broadcast_to(hn_ref[pl.ds(i1, 1), :], (16, D)),
                   jnp.broadcast_to(hn_ref[pl.ds(i2, 1), :], (16, D))).astype(BF16)
    for i in range(4, 7):
        w_copy(i).wait()
    gg = jnp.dot(xs, wg_ref[...], preferred_element_type=F32)
    uu = jnp.dot(xs, wu_ref[...], preferred_element_type=F32)
    act = (gg * jax.nn.sigmoid(gg) * uu).astype(BF16)
    yy = jnp.dot(act, wd_ref[...], preferred_element_type=F32)
    rs = jnp.where(rowi == 0, m1, m2)
    yy = yy * jax.nn.sigmoid(rs)
    y1 = jnp.broadcast_to(yy[0:1], (16, D))
    y2 = jnp.broadcast_to(yy[1:2], (16, D))

    for c in range(NQ):
        o_copy(c).wait()

    def patch(idx_row, sem):
        base = pl.multiple_of((idx_row // 16) * 16, 16)
        rr = rowi + base
        blk = z_ref[pl.ds(base, 16), :]
        blk = blk + jnp.where(rr == i1, y1, 0.0) + jnp.where(rr == i2, y2, 0.0)
        y_ref[pl.ds(base, 16), :] = blk.astype(BF16)
        cp = pltpu.make_async_copy(y_ref.at[pl.ds(base, 16)], out_hbm.at[pl.ds(base, 16)], sem)
        cp.start()
        cp.wait()

    patch(i1, sem_o.at[0])
    patch(i2, sem_o.at[1])


@jax.jit
def pallas_sequential_preLN__mha_block__moe_arch_mod__prompt_kernel(
    A_x: jax.Array,
    A_wqkv: jax.Array,
    A_wo: jax.Array,
    B_x: jax.Array,
    B_w_r: jax.Array,
    B_w_gate: jax.Array,
    B_w_up: jax.Array,
    B_w_down: jax.Array,
):
    del B_x
    x = A_x.reshape(S, D)
    wr = B_w_r.reshape(1, D)
    anyspec = pl.BlockSpec(memory_space=pl.ANY)
    out = pl.pallas_call(
        _kernel,
        out_shape=jax.ShapeDtypeStruct((S, D), BF16),
        in_specs=[anyspec, anyspec, anyspec, pl.BlockSpec(memory_space=pltpu.VMEM),
                  anyspec, anyspec, anyspec],
        out_specs=anyspec,
        scratch_shapes=[
            pltpu.VMEM((S, D), BF16),
            pltpu.VMEM((D, D), BF16),
            pltpu.VMEM((D, D), BF16),
            pltpu.VMEM((D, D), BF16),
            pltpu.VMEM((S // 2, D), U32),
            pltpu.VMEM((S // 2, D), U32),
            pltpu.VMEM((D, D), BF16),
            pltpu.VMEM((D, FF), BF16),
            pltpu.VMEM((D, FF), BF16),
            pltpu.VMEM((FF, D), BF16),
            pltpu.VMEM((D, D), BF16),
            pltpu.VMEM((D, D), BF16),
            pltpu.VMEM((NG, S // 2, 128), U32),
            pltpu.VMEM((NG, NC * OFF, 128), F32),
            pltpu.VMEM((NG * NQ, 64, TQ), U32),
            pltpu.VMEM((NG * NQ, 128, TQ), F32),
            pltpu.VMEM((NG, 64, S), U32),
            pltpu.VMEM((NG * NQ, 128, TQ), BF16),
            pltpu.VMEM((1, DH, TQ), F32),
            pltpu.VMEM((S, D), F32),
            pltpu.VMEM((S, D), F32),
            pltpu.VMEM((S, D), BF16),
            pltpu.VMEM((8, S), F32),
        ] + [pltpu.VMEM((1, CK // 2, TQ), U32)] * NPB + [
            pltpu.SemaphoreType.DMA((NQ,)),
            pltpu.SemaphoreType.DMA((7,)),
            pltpu.SemaphoreType.DMA((NQ,)),
        ],
        compiler_params=pltpu.CompilerParams(vmem_limit_bytes=100 * 1024 * 1024),
    )(x, A_wqkv, A_wo, wr, B_w_gate, B_w_up, B_w_down)
    return out.reshape(1, S, D)
```

```python
import functools
import math

import jax
import jax.numpy as jnp
from jax import lax
from jax.experimental import pallas as pl
from jax.experimental.pallas import tpu as pltpu

F32 = jnp.float32
BF16 = jnp.bfloat16
U32 = jnp.uint32

S = 2048
D = 512
H = 32
DH = 16
FF = 1792
TQ = 512
CK = 128
NQ = S // TQ
NC = S // CK
NL = TQ // 128
NG = D // 128
OFF = 16
MR = CK - OFF
LAG = 2
NPB = LAG + 2
EPS = 1e-5
OP = (0, 512, 1024, 1536, 2048)
XP = (0, 256, 512, 1024, 1536, 2048)
P1 = "X0.W0.X1.X2.W1.W2.X3.X4.x0.l0.w0.x1.k0.l1.k1.x2.w1.t0.q0.l2.k2.w2.x3.x4.W3.W7.W4.W5.W6.q1.u0.l3.v0.l4.v1.k3.q2.v2.k4.q3.v3"
QSCALE = (DH ** -0.5) * math.log2(math.e)
NEG = -3.0e38
SAFE_SCORE = 96.0
SAFE_V = 65536.0
PSP, PGR, POF = (8, 2, 0)
CARRY = 0
PAD = 0
VDEP, NPH, PSH = (2, 8, 7)


def _pk(x):
    return pltpu.bitcast(x, U32)


def _upk(x):
    return pltpu.bitcast(x, BF16)


def _layernorm(x):
    m = jnp.mean(x, axis=-1, keepdims=True)
    xc = x - m
    v = jnp.mean(xc * xc, axis=-1, keepdims=True)
    return xc * lax.rsqrt(v + EPS)


def _absmax8(x):
    r, c = x.shape
    a = jnp.abs(x).reshape(r // 8, 8, c).max(axis=0)
    out = a[:, 0:128]
    for t in range(1, c // 128):
        out = jnp.maximum(out, a[:, t * 128:(t + 1) * 128])
    return out


def _kernel(x_hbm, wqkv_hbm, wo_hbm, wr_hbm, wg_hbm, wu_hbm, wd_hbm, out_hbm,
            x_ref, wr_ref, wq_ref, wk_ref, wv_ref, xb_ref, xi_ref, wo_ref, wg_ref, wu_ref, wd_ref,
            wqt_ref, wvt_ref, k_ref, kf_ref, qt_ref, qf_ref, vt_ref, ot_ref,
            acc_ref, inv_ref, hn_ref, z_ref, y_ref, r_ref,
            p0, p1, p2, p3, sem_x, sem_w, sem_o):
    p_refs = (p0, p1, p2, p3)

    def x_copy(c):
        r0, r1 = XP[c], XP[c + 1]
        return pltpu.make_async_copy(x_hbm.at[pl.ds(r0, r1 - r0)], x_ref.at[pl.ds(r0, r1 - r0)], sem_x.at[c])

    def w_copy(i):
        src, dst = ((wqkv_hbm.at[:, pl.ds(D, D)], wk_ref), (wqkv_hbm.at[:, pl.ds(0, D)], wq_ref),
                    (wqkv_hbm.at[:, pl.ds(2 * D, D)], wv_ref), (wo_hbm, wo_ref), (wg_hbm, wg_ref),
                    (wu_hbm, wu_ref), (wd_hbm, wd_ref), (wr_hbm, wr_ref))[i]
        return pltpu.make_async_copy(src, dst, sem_w.at[i])

    def o_copy(c):
        r0, r1 = OP[c], OP[c + 1]
        return pltpu.make_async_copy(y_ref.at[pl.ds(r0, r1 - r0)], out_hbm.at[pl.ds(r0, r1 - r0)], sem_o.at[c])

    nt = (((1,), (1,)), ((), ()))
    mx = {}

    def upd(name, v):
        mx[name] = jnp.maximum(mx[name], v) if name in mx else v

    def ln1(c):
        r0, r1 = XP[c], XP[c + 1]
        xn = _layernorm(x_ref[r0:r1, :].astype(F32))
        xb_ref[r0 // 2:r1 // 2, :] = _pk(xn.astype(BF16))
        x4 = xn.reshape((r1 - r0) // 16, 2, 8, D)
        xi_ref[r0 // 2:r1 // 2, :] = pltpu.pack_elementwise(
            [x4[:, 0], x4[:, 1]], packed_dtype=BF16).reshape((r1 - r0) // 2, D)

    def kproj(c):
        r0, r1 = XP[c], XP[c + 1]
        xb = _upk(xb_ref[r0 // 2:r1 // 2, :])
        kb = jnp.dot(xb, wk_ref[...], preferred_element_type=F32).astype(BF16)
        kf = kb.astype(F32)
        ku = _pk(kb)
        for g in range(NG):
            k_ref[g, r0 // 2:r1 // 2, :] = ku[:, g * 128:(g + 1) * 128]
            for cc in range((r1 - r0) // CK):
                row = (r0 // CK + cc) * OFF
                kf_ref[0, g, row:row + OFF, :] = kf[cc * CK + MR:(cc + 1) * CK, g * 128:(g + 1) * 128]
        upd('k', _absmax8(kf))

    def qproj(c):
        xb = _upk(xb_ref[c * TQ // 2:(c + 1) * TQ // 2, :])
        qb = (lax.dot_general(wqt_ref[...], xb, nt, preferred_element_type=F32) * QSCALE).astype(BF16)
        qf = qb.astype(F32)
        qu = _pk(qb)
        for g in range(NG):
            qt_ref[g * NQ + c] = qu[g * 64:(g + 1) * 64, :]
            qf_ref[g * NQ + c] = qf[g * 128:(g + 1) * 128, :]
        qa = jnp.abs(qf).reshape(H, 2, 8, TQ)
        upd('q', _absmax8(jnp.sum(qa[:, 0] + qa[:, 1], axis=1)))

    def vproj(c):
        xi = _upk(xi_ref[c * TQ // 2:(c + 1) * TQ // 2, :])
        vb = lax.dot_general(wvt_ref[...], xi, nt, preferred_element_type=F32).astype(BF16)
        vu = _pk(vb)
        for g in range(NG):
            vt_ref[g, :, c * TQ:(c + 1) * TQ] = vu[g * 64:(g + 1) * 64, :]
        upd('v', _absmax8(vb.astype(F32)))

    def tq(_):
        wqt_ref[...] = wq_ref[...].astype(F32).T.astype(BF16)

    def tv(_):
        wvt_ref[...] = wv_ref[...].astype(F32).T.astype(BF16)

    acts = dict(X=lambda c: x_copy(c).start(), W=lambda c: w_copy(c).start(), x=lambda c: x_copy(c).wait(),
                w=lambda c: w_copy(c).wait(), l=ln1, k=kproj, q=qproj, v=vproj, t=tq, u=tv)
    for tok in P1.split("."):
        acts[tok[0]](int(tok[1:]))
    qmax, kmax, vmax = mx['q'], mx['k'], mx['v']

    bound = jnp.max(qmax) * jnp.max(kmax)
    safe = jnp.logical_and(bound <= SAFE_SCORE, jnp.max(vmax) <= SAFE_V)

    def pv_chunk(st, z0, z1, i, g, j, c, slot, n):
        pops = st.get(('pops', n + LAG - 1))
        parts = [None] * 8
        for q, r in enumerate(range(7, -1, -1)):
            if q % PGR == 0 and pops is not None:
                p_refs[slot][z0, CK // 2:CK // 2 + 8, 0:128] = _pk(pops[min(POF + (q * PSP) // 8, len(pops) - 1)])
            parts[r] = p_refs[slot][z1, r * 8:(r + 1) * 8, :]
        pw = jnp.concatenate(parts, axis=0)
        a = jnp.dot(_upk(vt_ref[g, j * 8:(j + 1) * 8, c * CK:(c + 1) * CK]), _upk(pw),
                    preferred_element_type=F32)
        acc = a if c == 0 else acc_ref[z1] + a
        if c < NC - 1:
            acc_ref[z0] = acc
        else:
            inv = inv_ref[...] if n < 0 else st['inv', j]
            ot_ref[i, j * DH:(j + 1) * DH, :] = (acc * inv).astype(BF16)

    def fast_body(i, carry):
        g = i // NQ
        z0 = i >> 8
        z1 = i >> 9
        st = {}
        deps = [None] * (VDEP * NPH)

        def qk(j, c, slot, n):
            def emit(r, a, b, key):
                pa = jnp.exp2(a)
                pb = jnp.exp2(b)
                p_refs[slot][z0, r * 8:(r + 1) * 8, :] = pltpu.pack_elementwise([pa, pb], packed_dtype=BF16)
                t = pa + pb
                st[key] = t if st[key] is None else st[key] + t

            if c == 0:
                st['l'] = None
                st['l2'] = None

            z = jnp.zeros((8, TQ), U32)
            qm = jnp.concatenate([z] * j + [qt_ref[i, j * 8:(j + 1) * 8, :]] + [z] * (7 - j), axis=0)
            kc = _upk(k_ref[g, c * CK // 2:c * CK // 2 + MR // 2, :])
            s = jnp.dot(kc, _upk(qm), preferred_element_type=F32)
            for ph in range(NPH):
                rr = (ph * (MR // 8) // NPH) * 8
                deps.append(s[rr:rr + 8, 0:128])
            st['pops', n] = [s[r * 8:(r + 1) * 8, 0:128] for r in range(MR // 8)]
            for r in range(MR // 16):
                emit(r, s[r * 16:r * 16 + 8], s[r * 16 + 8:r * 16 + 16], 'l')

            accs = [[None] * NL for _ in range(2)]
            for d in range(DH):
                if d % (DH // NPH) == 0:
                    dep = deps[n * NPH + d // (DH // NPH) + PSH]
                    if dep is not None:
                        kf_ref[z0, NG, 0:8, :] = dep
                    if dep is not None or d == 0:
                        kfs = [kf_ref[z1, g, c * OFF + r * 8:c * OFF + (r + 1) * 8, :] for r in range(2)]
                kbs = [jnp.broadcast_to(kf[:, j * DH + d:j * DH + d + 1], (8, 128)) for kf in kfs]
                for t in range(NL):
                    qv = jnp.broadcast_to(qf_ref[i, j * DH + d:j * DH + d + 1, t * 128:(t + 1) * 128], (8, 128))
                    for r in range(2):
                        x = kbs[r] * qv
                        accs[r][t] = x if accs[r][t] is None else accs[r][t] + x
            emit(MR // 16, jnp.concatenate(accs[0], axis=1), jnp.concatenate(accs[1], axis=1), 'l2')
            if c == NC - 1:
                st['inv', j] = 1.0 / jnp.sum(st['l'] + st['l2'], axis=0, keepdims=True)

        pv = functools.partial(pv_chunk, st, z0, z1)
        ip = lax.rem(i + NG * NQ, NG * NQ + 1)
        gp = lax.rem(i + NG * NQ - 1, NG * NQ) // NQ
        pend = [(ip, gp, 7, NC - LAG + q, (q - LAG) % NPB, q - LAG) for q in range(LAG)]
        pend = pend[LAG - CARRY:]
        n = 0
        for j in range(8):
            for c in range(NC):
                slot = n % NPB
                qk(j, c, slot, n)
                pend.append((i, g, j, c, slot, n))
                n += 1
                if len(pend) > LAG or (pend[0][-1] < 0 and pend[0][-1] + LAG < n):
                    pv(*pend.pop(0))
        st['pops', n] = st['pops', n - 1]
        for item in pend[:LAG - CARRY]:
            pv(*item)
        inv_ref[...] = st['inv', 7]
        return carry

    def slow_body(t, carry):
        i = t // 8
        j = t % 8
        g = i // NQ
        rows = lax.broadcasted_iota(jnp.int32, (64, TQ), 0)
        qm = _upk(jnp.where(rows // 8 == j, qt_ref[i], jnp.zeros((64, TQ), U32)))

        def scores(c):
            kc = _upk(k_ref[g, pl.ds(pl.multiple_of(c * (CK // 2), CK // 2), CK // 2), :])
            return jnp.dot(kc, qm, preferred_element_type=F32)

        def max_body(c, m):
            return jnp.maximum(m, jnp.max(scores(c), axis=0, keepdims=True))

        m = lax.fori_loop(0, NC, max_body, jnp.full((1, TQ), -jnp.inf, F32))
        vrow = pl.multiple_of(j * 8, 8)

        def acc_body(c, carry):
            acc, l = carry
            p = jnp.exp2(scores(c) - m)
            p4 = p.reshape(CK // 16, 2, 8, TQ)
            pp = _upk(pltpu.pack_elementwise([p4[:, 0], p4[:, 1]], packed_dtype=BF16).reshape(CK // 2, TQ))
            vc = _upk(vt_ref[g, pl.ds(vrow, 8), pl.ds(pl.multiple_of(c * CK, CK), CK)])
            return (acc + jnp.dot(vc, pp, preferred_element_type=F32),
                    l + jnp.sum(p, axis=0, keepdims=True))

        acc, l = lax.fori_loop(0, NC, acc_body, (jnp.zeros((DH, TQ), F32), jnp.zeros((1, TQ), F32)))
        ot_ref[i, pl.ds(pl.multiple_of(j * DH, DH), DH), :] = (acc / l).astype(BF16)
        return carry

    @pl.when(safe)
    def _():
        for q in range(LAG):
            p_refs[(q - LAG) % NPB][...] = jnp.zeros(p0.shape, U32)
        acc_ref[...] = jnp.zeros(acc_ref.shape, F32)
        inv_ref[...] = jnp.zeros(inv_ref.shape, F32)
        lax.fori_loop(0, 16, fast_body, 0)
        for q in range(LAG - CARRY, LAG):
            pv_chunk({}, 0, 0, NG * NQ - 1, NG - 1, 7, NC - LAG + q, (q - LAG) % NPB, q - LAG)

    @pl.when(jnp.logical_not(safe))
    def _():
        lax.fori_loop(0, NG * NQ * 8, slow_body, 0)

    w_copy(3).wait()
    w_copy(7).wait()
    tn = (((0,), (0,)), ((), ()))
    wr8 = jnp.broadcast_to(wr_ref[...].astype(F32).reshape(1, D), (16, D)).astype(BF16)
    TR = 128
    NR = S // TR

    XT = 2

    def otrans(c):
        qb, off = divmod(c * TR, TQ)
        ot = jnp.concatenate([ot_ref[g * NQ + qb, :, off:off + TR] for g in range(NG)], axis=0)
        xb_ref[c * TR // 2:(c + 1) * TR // 2, :] = _pk(ot.T)

    def oproj(c):
        qb, off = divmod(c * TR, TQ)
        if XT:
            if c == 0:
                for cc in range(XT):
                    otrans(cc)
            if c + XT < NR:
                otrans(c + XT)
            a = jnp.dot(_upk(xb_ref[c * TR // 2:(c + 1) * TR // 2, :]), wo_ref[...], preferred_element_type=F32)
        else:
            ot = jnp.concatenate([ot_ref[g * NQ + qb, :, off:off + TR] for g in range(NG)], axis=0)
            a = lax.dot_general(ot, wo_ref[...], tn, preferred_element_type=F32)
        z_ref[c * TR:(c + 1) * TR, :] = x_ref[c * TR:(c + 1) * TR, :].astype(F32) + a

    def ln2(c):
        h = z_ref[c * TR:(c + 1) * TR, :]
        hn = _layernorm(h)
        zz = h + hn
        hn_ref[c * TR:(c + 1) * TR, :] = hn
        z_ref[c * TR:(c + 1) * TR, :] = zz
        y_ref[c * TR:(c + 1) * TR, :] = zz.astype(BF16)

    def router(c0, c1):
        hb = hn_ref[c0 * TR:c1 * TR, :].astype(BF16)
        r = lax.dot_general(wr8, hb, nt, preferred_element_type=F32)
        r_ref[:, c0 * TR:c1 * TR] = r[0:8].astype(BF16).astype(F32)

    AH = 1
    RB = 1
    for c in range(AH):
        oproj(c)
    done = 0
    for c in range(NR):
        if c + AH < NR:
            oproj(c + AH)
        if c - done >= RB:
            router(done, c)
            done = c
        ln2(c)
        if c + 1 == NR:
            router(done, NR)
        if (c + 1) * TR in OP[1:]:
            o_copy(OP.index((c + 1) * TR) - 1).start()

    rb = pltpu.bitcast(r_ref[...], jnp.int32)
    rb = jnp.where(rb < 0, jnp.int32(-2147483648) - rb, rb)
    idx = lax.broadcasted_iota(jnp.int32, (8, S), 1)
    key = rb + (S - 1 - idx)
    k1 = jnp.max(key)
    k2 = jnp.max(jnp.where(key == k1, jnp.int32(-2147483648), key))
    i1 = jnp.clip((S - 1) - (k1 & 0xFFFF), 0, S - 1)
    i2 = jnp.clip((S - 1) - (k2 & 0xFFFF), 0, S - 1)
    rowi = lax.broadcasted_iota(jnp.int32, (16, D), 0)
    xs = jnp.where(rowi == 0, jnp.broadcast_to(hn_ref[pl.ds(i1, 1), :], (16, D)),
                   jnp.broadcast_to(hn_ref[pl.ds(i2, 1), :], (16, D))).astype(BF16)
    ks = jnp.where(rowi == 0, k1, k2) & jnp.int32(-65536)
    rs = pltpu.bitcast(jnp.where(ks < 0, jnp.int32(-2147483648) - ks, ks), F32)
    for i in range(4, 7):
        w_copy(i).wait()
    gg = jnp.dot(xs, wg_ref[...], preferred_element_type=F32)
    uu = jnp.dot(xs, wu_ref[...], preferred_element_type=F32)
    act = (gg * jax.nn.sigmoid(gg) * uu).astype(BF16)
    yy = jnp.dot(act, wd_ref[...], preferred_element_type=F32)
    yy = yy * jax.nn.sigmoid(rs)
    y1 = jnp.broadcast_to(yy[0:1], (16, D))
    y2 = jnp.broadcast_to(yy[1:2], (16, D))

    for c in range(len(OP) - 1):
        o_copy(c).wait()

    def patch(base):
        rr = rowi + base
        blk = z_ref[pl.ds(base, 16), :]
        blk = blk + jnp.where(rr == i1, y1, 0.0) + jnp.where(rr == i2, y2, 0.0)
        y_ref[pl.ds(base, 16), :] = blk.astype(BF16)

    def patch_copy(base, sem):
        return pltpu.make_async_copy(y_ref.at[pl.ds(base, 16)], out_hbm.at[pl.ds(base, 16)], sem)

    b1 = pl.multiple_of((i1 >> 4) << 4, 16)
    b2 = pl.multiple_of((i2 >> 4) << 4, 16)
    patch(b1)
    patch(b2)
    patch_copy(b1, sem_o.at[0]).start()

    @pl.when(b1 != b2)
    def _():
        cp = patch_copy(b2, sem_o.at[1])
        cp.start()
        cp.wait()

    patch_copy(b1, sem_o.at[0]).wait()


@jax.jit
def pallas_sequential_preLN__mha_block__moe_arch_mod__prompt_kernel(
    A_x: jax.Array,
    A_wqkv: jax.Array,
    A_wo: jax.Array,
    B_x: jax.Array,
    B_w_r: jax.Array,
    B_w_gate: jax.Array,
    B_w_up: jax.Array,
    B_w_down: jax.Array,
):
    del B_x
    x = A_x.reshape(S, D)
    wr = B_w_r
    anyspec = pl.BlockSpec(memory_space=pl.ANY)
    out = pl.pallas_call(
        _kernel,
        out_shape=jax.ShapeDtypeStruct((S, D), BF16),
        in_specs=[anyspec] * 7,
        out_specs=anyspec,
        scratch_shapes=[
            pltpu.VMEM((S, D), BF16),
            pltpu.VMEM((D,), BF16),
            pltpu.VMEM((D, D), BF16),
            pltpu.VMEM((D, D), BF16),
            pltpu.VMEM((D, D), BF16),
            pltpu.VMEM((S // 2, D), U32),
            pltpu.VMEM((S // 2, D), U32),
            pltpu.VMEM((D, D), BF16),
            pltpu.VMEM((D, FF), BF16),
            pltpu.VMEM((D, FF), BF16),
            pltpu.VMEM((FF, D), BF16),
            pltpu.VMEM((D, D), BF16),
            pltpu.VMEM((D, D), BF16),
            pltpu.VMEM((NG, S // 2, 128), U32),
            pltpu.VMEM((1, NG + 1, NC * OFF, 128), F32),
            pltpu.VMEM((NG * NQ, 64, TQ), U32),
            pltpu.VMEM((NG * NQ, 128, TQ), F32),
            pltpu.VMEM((NG, 64, S), U32),
            pltpu.VMEM((NG * NQ + 1, 128, TQ), BF16),
            pltpu.VMEM((1, DH, TQ), F32),
            pltpu.VMEM((1, TQ), F32),
            pltpu.VMEM((S, D), F32),
            pltpu.VMEM((S, D), F32),
            pltpu.VMEM((S, D), BF16),
            pltpu.VMEM((8, S), F32),
        ] + [pltpu.VMEM((1, CK // 2 + 8, TQ), U32)] * NPB + [
            pltpu.SemaphoreType.DMA((8,)),
            pltpu.SemaphoreType.DMA((8,)),
            pltpu.SemaphoreType.DMA((NQ,)),
        ],
        compiler_params=pltpu.CompilerParams(vmem_limit_bytes=100 * 1024 * 1024),
    )(x, A_wqkv, A_wo, wr, B_w_gate, B_w_up, B_w_down)
    return out.reshape(1, S, D)
```

```python
import math

import jax
import jax.numpy as jnp
from jax import lax
from jax.experimental import pallas as pl
from jax.experimental.pallas import tpu as pltpu

F32 = jnp.float32
BF16 = jnp.bfloat16
U32 = jnp.uint32
I32 = jnp.int32

S = 2048
D = 512
H = 32
DH = 16
FF = 1792
TQ = 512
CK = 128
NQ = S // TQ
NC = S // CK
NL = TQ // 128
NG = D // 128
OFF = 16
MR = CK - OFF
LAG = 2
NPB = 4
NB = 2
TR = 128
XP = (0, 256, 512, 1024, 1536, 2048)
EPS = 1e-5
QSCALE = (DH ** -0.5) * math.log2(math.e)
INT_MIN = -2 ** 31
SAFE_SCORE = 96.0
SAFE_V = 65536.0
VDEP, NPH, PSH = (2, 8, 7)
PSP, PGR = (8, 2)
DT1 = 2
P1LOOP = 1


def _pk(x):
    return pltpu.bitcast(x, U32)


def _upk(x):
    return pltpu.bitcast(x, BF16)


def _ds(start, size):
    if isinstance(start, int):
        return pl.ds(start, size)
    return pl.ds(pl.multiple_of(start, size), size)


def _pack_pairs(x):
    r, c = x.shape
    x4 = x.reshape(r // 16, 2, 8, c)
    return pltpu.pack_elementwise([x4[:, 0], x4[:, 1]], packed_dtype=BF16).reshape(r // 2, c)


def _layernorm(x):
    m = jnp.mean(x, axis=-1, keepdims=True)
    xc = x - m
    v = jnp.mean(xc * xc, axis=-1, keepdims=True)
    return xc * lax.rsqrt(v + EPS)


def _absmax8(x):
    r, c = x.shape
    a = jnp.abs(x).reshape(r // 8, 8, c).max(axis=0)
    out = a[:, 0:128]
    for t in range(1, c // 128):
        out = jnp.maximum(out, a[:, t * 128:(t + 1) * 128])
    return out


def _kernel(x_hbm, wqkv_hbm, wo_hbm, wr_hbm, wg_hbm, wu_hbm, wd_hbm, out_hbm,
            x_ref, wr_ref, wq_ref, wk_ref, wv_ref, wo_ref, wg_ref, wu_ref, wd_ref,
            xb_ref, xi_ref, wqt_ref, wvt_ref, k_ref, kf_ref, qt_ref, qf_ref, vt_ref, ot_ref,
            acc_ref, hn_ref, z_ref, y_ref, r_ref, p0, p1, p2, p3, sem_x, sem_w, sem_o):
    p_refs = (p0, p1, p2, p3)
    nt = (((1,), (1,)), ((), ()))

    def x_copy(c):
        rows = pl.ds(XP[c], XP[c + 1] - XP[c])
        return pltpu.make_async_copy(x_hbm.at[rows], x_ref.at[rows], sem_x.at[c])

    def w_copy(i):
        src, dst = ((wqkv_hbm.at[:, pl.ds(D, D)], wk_ref), (wqkv_hbm.at[:, pl.ds(0, D)], wq_ref),
                    (wqkv_hbm.at[:, pl.ds(2 * D, D)], wv_ref), (wo_hbm, wo_ref), (wr_hbm, wr_ref),
                    (wg_hbm, wg_ref), (wu_hbm, wu_ref), (wd_hbm, wd_ref))[i]
        return pltpu.make_async_copy(src, dst, sem_w.at[i])

    def o_copy(c):
        rows = pl.ds(c * TQ, TQ)
        return pltpu.make_async_copy(y_ref.at[rows], out_hbm.at[rows], sem_o.at[c])

    def ln1(c):
        r0, r1 = XP[c], XP[c + 1]
        xn = _layernorm(x_ref[r0:r1, :].astype(F32))
        xb_ref[r0 // 2:r1 // 2, :] = _pk(xn.astype(BF16))
        xi_ref[r0 // 2:r1 // 2, :] = _pack_pairs(xn)

    def kproj(r0, n):
        xb = _upk(xb_ref[_ds(r0 // 2, n // 2), :])
        kb = jnp.dot(xb, wk_ref[...], preferred_element_type=F32).astype(BF16)
        kf = kb.astype(F32)
        ku = _pk(kb)
        for g in range(NG):
            k_ref[g, _ds(r0 // 2, n // 2), :] = ku[:, g * 128:(g + 1) * 128]
            for cc in range(n // CK):
                kf_ref[0, g, _ds((r0 // CK + cc) * OFF, OFF), :] = kf[cc * CK + MR:(cc + 1) * CK,
                                                                      g * 128:(g + 1) * 128]
        return _absmax8(kf)

    def qproj(c):
        xb = _upk(xb_ref[_ds(c * (TQ // 2), TQ // 2), :])
        qb = (lax.dot_general(wqt_ref[...], xb, nt, preferred_element_type=F32) * QSCALE).astype(BF16)
        qf = qb.astype(F32)
        qu = _pk(qb)
        for g in range(NG):
            qt_ref[g * NQ + c] = qu[g * 64:(g + 1) * 64, :]
            qf_ref[g * NQ + c] = qf[g * 128:(g + 1) * 128, :]
        qa = jnp.abs(qf).reshape(H, 2, 8, TQ)
        return _absmax8(jnp.sum(qa[:, 0] + qa[:, 1], axis=1))

    def vproj(c):
        xi = _upk(xi_ref[_ds(c * (TQ // 2), TQ // 2), :])
        vb = lax.dot_general(wvt_ref[...], xi, nt, preferred_element_type=F32).astype(BF16)
        vu = _pk(vb)
        for g in range(NG):
            vt_ref[g, :, _ds(c * TQ, TQ)] = vu[g * 64:(g + 1) * 64, :]
        return _absmax8(vb.astype(F32))

    x_copy(0).start()
    w_copy(0).start()
    x_copy(1).start()
    x_copy(2).start()
    w_copy(1).start()
    w_copy(2).start()
    x_copy(3).start()
    x_copy(4).start()
    x_copy(0).wait()
    ln1(0)
    w_copy(0).wait()
    x_copy(1).wait()
    km = kproj(0, 256)
    ln1(1)
    km = jnp.maximum(km, kproj(256, 256))
    x_copy(2).wait()
    w_copy(1).wait()
    wqt_ref[...] = wq_ref[...].astype(F32).T.astype(BF16)
    qm = qproj(0)
    ln1(2)
    km = jnp.maximum(km, kproj(TQ, TQ))
    w_copy(2).wait()
    x_copy(3).wait()
    x_copy(4).wait()
    for i in range(3, 8):
        w_copy(i).start()
    qm = jnp.maximum(qm, qproj(1))
    wvt_ref[...] = wv_ref[...].astype(F32).T.astype(BF16)
    ln1(3)
    vm = vproj(0)
    ln1(4)
    vm = jnp.maximum(vm, vproj(1))

    def proj_body(c, carry):
        km, qm, vm = carry
        return (jnp.maximum(km, kproj(c * TQ, TQ)), jnp.maximum(qm, qproj(c)), jnp.maximum(vm, vproj(c)))

    if P1LOOP:
        km, qm, vm = lax.fori_loop(2, NQ, proj_body, (km, qm, vm))
    else:
        for c in range(2, NQ):
            km, qm, vm = proj_body(c, (km, qm, vm))

    safe = jnp.logical_and(jnp.max(qm) * jnp.max(km) <= SAFE_SCORE, jnp.max(vm) <= SAFE_V)

    def fast_body(it, carry):
        z0 = it >> 8
        z1 = it >> 9
        st = {}
        deps = [None] * (VDEP * NPH)

        blk = [it * NB + b for b in range(NB)]
        grp = [i // NQ for i in blk]

        def qk(b, j, c, n):
            i, g = blk[b], grp[b]
            p_ref = p_refs[n % NPB]

            def emit(r, a, b_, key):
                pa = jnp.exp2(a)
                pb = jnp.exp2(b_)
                p_ref[z0, r * 8:(r + 1) * 8, :] = pltpu.pack_elementwise([pa, pb], packed_dtype=BF16)
                t = pa + pb
                st[key] = t if st[key] is None else st[key] + t

            if c == 0:
                st['l'] = None
                st['l2'] = None

            z = jnp.zeros((8, TQ), U32)
            qm = jnp.concatenate([z] * j + [qt_ref[i, j * 8:(j + 1) * 8, :]] + [z] * (7 - j), axis=0)
            order = list(range(MR // 16))[::-1]
            kc = _upk(jnp.concatenate(
                [k_ref[g, c * CK // 2 + r * 8:c * CK // 2 + (r + 1) * 8, :] for r in order], axis=0))
            s = jnp.dot(kc, _upk(qm), preferred_element_type=F32)
            for ph in range(NPH):
                rr = (ph * (MR // 8) // NPH) * 8
                deps.append(s[rr:rr + 8, DT1 * 128:(DT1 + 1) * 128])
            st['pops', n] = [s[r * 8:(r + 1) * 8, 0:128] for r in range(MR // 8)]
            for q, r in enumerate(order):
                emit(r, s[q * 16:q * 16 + 8], s[q * 16 + 8:q * 16 + 16], 'l')

            accs = [[None] * NL for _ in range(2)]
            for d in range(DH):
                if d % (DH // NPH) == 0:
                    dep = deps[n * NPH + d // (DH // NPH) + PSH]
                    if dep is not None:
                        kf_ref[z0, NG, 0:8, :] = dep
                    if dep is not None or d == 0:
                        kfs = [kf_ref[z1, g, c * OFF + r * 8:c * OFF + (r + 1) * 8, :] for r in range(2)]
                kbs = [jnp.broadcast_to(kf[:, j * DH + d:j * DH + d + 1], (8, 128)) for kf in kfs]
                for t in range(NL):
                    qv = jnp.broadcast_to(qf_ref[i, j * DH + d:j * DH + d + 1, t * 128:(t + 1) * 128], (8, 128))
                    for r in range(2):
                        x = kbs[r] * qv
                        accs[r][t] = x if accs[r][t] is None else accs[r][t] + x
            emit(MR // 16, jnp.concatenate(accs[0], axis=1), jnp.concatenate(accs[1], axis=1), 'l2')
            if c == NC - 1:
                st['inv', b, j] = 1.0 / jnp.sum(st['l'] + st['l2'], axis=0, keepdims=True)

        def pv(b, j, c, n):
            p_ref = p_refs[n % NPB]
            pops = st['pops', min(n + LAG, len(work)) - 1]
            parts = [None] * 8
            for q, r in enumerate(range(7, -1, -1)):
                if q % PGR == 0:
                    p_ref[z0, CK // 2:CK // 2 + 8, 0:128] = _pk(pops[(q * PSP) // 8])
                parts[r] = p_ref[z1, r * 8:(r + 1) * 8, :]
            a = jnp.dot(_upk(vt_ref[grp[b], j * 8:(j + 1) * 8, c * CK:(c + 1) * CK]),
                        _upk(jnp.concatenate(parts, axis=0)), preferred_element_type=F32)
            acc = a if c == 0 else acc_ref[z1] + a
            if c < NC - 1:
                acc_ref[z0] = acc
            else:
                ot_ref[blk[b], j * DH:(j + 1) * DH, :] = (acc * st['inv', b, j]).astype(BF16)

        work = [(b, j, c) for b in range(NB) for j in range(8) for c in range(NC)]
        for n in range(len(work) + LAG):
            if n < len(work):
                qk(*work[n], n)
            if n >= LAG:
                pv(*work[n - LAG], n - LAG)
        return carry

    def slow_body(t, carry):
        i = t // 8
        j = t % 8
        g = i // NQ
        rows = lax.broadcasted_iota(I32, (64, TQ), 0)
        qm = _upk(jnp.where(rows // 8 == j, qt_ref[i], jnp.zeros((64, TQ), U32)))

        def scores(c):
            kc = _upk(k_ref[g, _ds(c * (CK // 2), CK // 2), :])
            return jnp.dot(kc, qm, preferred_element_type=F32)

        def max_body(c, m):
            return jnp.maximum(m, jnp.max(scores(c), axis=0, keepdims=True))

        m = lax.fori_loop(0, NC, max_body, jnp.full((1, TQ), -jnp.inf, F32))

        def acc_body(c, carry):
            acc, l = carry
            p = jnp.exp2(scores(c) - m)
            vc = _upk(vt_ref[g, _ds(j * 8, 8), _ds(c * CK, CK)])
            return (acc + jnp.dot(vc, _upk(_pack_pairs(p)), preferred_element_type=F32),
                    l + jnp.sum(p, axis=0, keepdims=True))

        acc, l = lax.fori_loop(0, NC, acc_body, (jnp.zeros((DH, TQ), F32), jnp.zeros((1, TQ), F32)))
        ot_ref[i, _ds(j * DH, DH), :] = (acc / l).astype(BF16)
        return carry

    @pl.when(safe)
    def _():
        lax.fori_loop(0, 16 // NB, fast_body, 0)

    @pl.when(jnp.logical_not(safe))
    def _():
        lax.fori_loop(0, NG * NQ * 8, slow_body, 0)

    w_copy(3).wait()
    w_copy(4).wait()
    wr16 = jnp.broadcast_to(wr_ref[...].astype(F32).reshape(1, D), (16, D)).astype(BF16)
    nr = S // TR

    def otrans(c):
        qb, off = divmod(c * TR, TQ)
        ot = jnp.concatenate([ot_ref[g * NQ + qb, :, off:off + TR] for g in range(NG)], axis=0)
        xb_ref[c * TR // 2:(c + 1) * TR // 2, :] = _pk(ot.T)

    def oproj(c):
        a = jnp.dot(_upk(xb_ref[c * TR // 2:(c + 1) * TR // 2, :]), wo_ref[...], preferred_element_type=F32)
        z_ref[c * TR:(c + 1) * TR, :] = x_ref[c * TR:(c + 1) * TR, :].astype(F32) + a

    def ln2(c):
        h = z_ref[c * TR:(c + 1) * TR, :]
        hn = _layernorm(h)
        zz = h + hn
        hn_ref[c * TR:(c + 1) * TR, :] = hn
        z_ref[c * TR:(c + 1) * TR, :] = zz
        y_ref[c * TR:(c + 1) * TR, :] = zz.astype(BF16)

    def router(c):
        hb = hn_ref[c * TR:(c + 1) * TR, :].astype(BF16)
        r = lax.dot_general(wr16, hb, nt, preferred_element_type=F32)
        r_ref[:, c * TR:(c + 1) * TR] = r[0:8].astype(BF16).astype(F32)

    for c in range(-3, nr + 1):
        if 0 <= c + 3 < nr:
            otrans(c + 3)
        if 0 <= c + 1 < nr:
            oproj(c + 1)
        if 0 <= c - 1 < nr:
            router(c - 1)
        if 0 <= c < nr:
            ln2(c)
            if ((c + 1) * TR) % TQ == 0:
                o_copy(((c + 1) * TR) // TQ - 1).start()

    rb = pltpu.bitcast(r_ref[...], I32)
    rb = jnp.where(rb < 0, INT_MIN - rb, rb)
    key = rb + (S - 1 - lax.broadcasted_iota(I32, (8, S), 1))
    k1 = jnp.max(key)
    k2 = jnp.max(jnp.where(key == k1, INT_MIN, key))
    i1 = jnp.clip((S - 1) - (k1 & 0xFFFF), 0, S - 1)
    i2 = jnp.clip((S - 1) - (k2 & 0xFFFF), 0, S - 1)
    rowi = lax.broadcasted_iota(I32, (16, D), 0)
    xs = jnp.where(rowi == 0, jnp.broadcast_to(hn_ref[pl.ds(i1, 1), :], (16, D)),
                   jnp.broadcast_to(hn_ref[pl.ds(i2, 1), :], (16, D))).astype(BF16)
    ks = jnp.where(rowi == 0, k1, k2) & -65536
    rs = pltpu.bitcast(jnp.where(ks < 0, INT_MIN - ks, ks), F32)
    for i in range(5, 8):
        w_copy(i).wait()
    gg = jnp.dot(xs, wg_ref[...], preferred_element_type=F32)
    uu = jnp.dot(xs, wu_ref[...], preferred_element_type=F32)
    act = (gg * jax.nn.sigmoid(gg) * uu).astype(BF16)
    yy = jnp.dot(act, wd_ref[...], preferred_element_type=F32) * jax.nn.sigmoid(rs)
    y1 = jnp.broadcast_to(yy[0:1], (16, D))
    y2 = jnp.broadcast_to(yy[1:2], (16, D))

    for c in range(NQ):
        o_copy(c).wait()

    def patch(base):
        rr = rowi + base
        blk = z_ref[pl.ds(base, 16), :]
        blk = blk + jnp.where(rr == i1, y1, 0.0) + jnp.where(rr == i2, y2, 0.0)
        y_ref[pl.ds(base, 16), :] = blk.astype(BF16)

    def patch_copy(base, sem):
        return pltpu.make_async_copy(y_ref.at[pl.ds(base, 16)], out_hbm.at[pl.ds(base, 16)], sem)

    b1 = pl.multiple_of((i1 >> 4) << 4, 16)
    b2 = pl.multiple_of((i2 >> 4) << 4, 16)
    patch(b1)
    patch(b2)
    patch_copy(b1, sem_o.at[0]).start()

    @pl.when(b1 != b2)
    def _():
        cp = patch_copy(b2, sem_o.at[1])
        cp.start()
        cp.wait()

    patch_copy(b1, sem_o.at[0]).wait()


@jax.jit
def pallas_sequential_preLN__mha_block__moe_arch_mod__prompt_kernel(
    A_x: jax.Array,
    A_wqkv: jax.Array,
    A_wo: jax.Array,
    B_x: jax.Array,
    B_w_r: jax.Array,
    B_w_gate: jax.Array,
    B_w_up: jax.Array,
    B_w_down: jax.Array,
):
    del B_x
    anyspec = pl.BlockSpec(memory_space=pl.ANY)
    out = pl.pallas_call(
        _kernel,
        out_shape=jax.ShapeDtypeStruct((S, D), BF16),
        in_specs=[anyspec] * 7,
        out_specs=anyspec,
        scratch_shapes=[
            pltpu.VMEM((S, D), BF16),
            pltpu.VMEM((D,), BF16),
            pltpu.VMEM((D, D), BF16),
            pltpu.VMEM((D, D), BF16),
            pltpu.VMEM((D, D), BF16),
            pltpu.VMEM((D, D), BF16),
            pltpu.VMEM((D, FF), BF16),
            pltpu.VMEM((D, FF), BF16),
            pltpu.VMEM((FF, D), BF16),
            pltpu.VMEM((S // 2, D), U32),
            pltpu.VMEM((S // 2, D), U32),
            pltpu.VMEM((D, D), BF16),
            pltpu.VMEM((D, D), BF16),
            pltpu.VMEM((NG, S // 2, 128), U32),
            pltpu.VMEM((1, NG + 1, NC * OFF, 128), F32),
            pltpu.VMEM((NG * NQ, 64, TQ), U32),
            pltpu.VMEM((NG * NQ, 128, TQ), F32),
            pltpu.VMEM((NG, 64, S), U32),
            pltpu.VMEM((NG * NQ, 128, TQ), BF16),
            pltpu.VMEM((1, DH, TQ), F32),
            pltpu.VMEM((S, D), F32),
            pltpu.VMEM((S, D), F32),
            pltpu.VMEM((S, D), BF16),
            pltpu.VMEM((8, S), F32),
        ] + [pltpu.VMEM((1, CK // 2 + 8, TQ), U32)] * NPB + [
            pltpu.SemaphoreType.DMA((len(XP) - 1,)),
            pltpu.SemaphoreType.DMA((8,)),
            pltpu.SemaphoreType.DMA((NQ,)),
        ],
        compiler_params=pltpu.CompilerParams(vmem_limit_bytes=100 * 1024 * 1024),
    )(A_x.reshape(S, D), A_wqkv, A_wo, B_w_r, B_w_gate, B_w_up, B_w_down)
    return out.reshape(1, S, D)
```

```python
import math

import jax
import jax.numpy as jnp
from jax import lax
from jax.experimental import pallas as pl
from jax.experimental.pallas import tpu as pltpu

F32 = jnp.float32
BF16 = jnp.bfloat16
U32 = jnp.uint32
I32 = jnp.int32

S = 2048
D = 512
H = 32
DH = 16
FF = 1792
TQ = 512
CK = 128
NQ = S // TQ
NC = S // CK
NL = TQ // 128
NG = D // 128
OFF = 16
MR = CK - OFF
LAG = 2
NPB = 4
NB = 2
TR = 128
WS = 256
XP = (0, 384, 512, 1024, 1536, 2048)
EPS = 1e-5
QSCALE = (DH ** -0.5) * math.log2(math.e)
INT_MIN = -2 ** 31
SAFE_SCORE = 96.0
SAFE_V = 65536.0
VDEP, NPH, PSH = (2, 8, 6)
PSP, PGR = (8, 2)
DT1 = 2
P1LOOP = 1


def _pk(x):
    return pltpu.bitcast(x, U32)


def _upk(x):
    return pltpu.bitcast(x, BF16)


def _ds(start, size):
    if isinstance(start, int):
        return pl.ds(start, size)
    return pl.ds(pl.multiple_of(start, size), size)


def _pack_pairs(x):
    r, c = x.shape
    x4 = x.reshape(r // 16, 2, 8, c)
    return pltpu.pack_elementwise([x4[:, 0], x4[:, 1]], packed_dtype=BF16).reshape(r // 2, c)


def _layernorm(x):
    m = jnp.mean(x, axis=-1, keepdims=True)
    xc = x - m
    v = jnp.mean(xc * xc, axis=-1, keepdims=True)
    return xc * lax.rsqrt(v + EPS)


def _absmax8(x):
    r, c = x.shape
    a = jnp.abs(x).reshape(r // 8, 8, c).max(axis=0)
    out = a[:, 0:128]
    for t in range(1, c // 128):
        out = jnp.maximum(out, a[:, t * 128:(t + 1) * 128])
    return out


def _kernel(x_hbm, wqkv_hbm, wo_hbm, wr_hbm, wg_hbm, wu_hbm, wd_hbm, out_hbm,
            x_ref, wr_ref, wq_ref, wk_ref, wv_ref, wo_ref, wg_ref, wu_ref, wd_ref,
            xb_ref, xi_ref, wqt_ref, wvt_ref, k_ref, kf_ref, qt_ref, qf_ref, vt_ref, ot_ref,
            acc_ref, hn_ref, z_ref, y_ref, p0, p1, p2, p3, sem_x, sem_w, sem_o):
    p_refs = (p0, p1, p2, p3)
    nt = (((1,), (1,)), ((), ()))

    def x_copy(c):
        rows = pl.ds(XP[c], XP[c + 1] - XP[c])
        return pltpu.make_async_copy(x_hbm.at[rows], x_ref.at[rows], sem_x.at[c])

    def w_copy(i):
        src, dst = ((wqkv_hbm.at[:, pl.ds(D, WS)], wk_ref.at[:, pl.ds(0, WS)]),
                    (wqkv_hbm.at[:, pl.ds(0, D)], wq_ref),
                    (wqkv_hbm.at[:, pl.ds(2 * D, D)], wv_ref), (wo_hbm, wo_ref), (wr_hbm, wr_ref),
                    (wg_hbm, wg_ref), (wu_hbm, wu_ref), (wd_hbm, wd_ref),
                    (wqkv_hbm.at[:, pl.ds(D + WS, D - WS)], wk_ref.at[:, pl.ds(WS, D - WS)]))[i]
        return pltpu.make_async_copy(src, dst, sem_w.at[i])

    def o_copy(c):
        rows = pl.ds(c * TQ, TQ)
        return pltpu.make_async_copy(y_ref.at[rows], out_hbm.at[rows], sem_o.at[c])

    def ln1(c):
        r0, r1 = XP[c], XP[c + 1]
        xn = _layernorm(x_ref[r0:r1, :].astype(F32))
        xb_ref[r0 // 2:r1 // 2, :] = _pk(xn.astype(BF16))
        xi_ref[r0 // 2:r1 // 2, :] = _pack_pairs(xn)

    def kproj(r0, n, g0=0, g1=NG):
        xb = _upk(xb_ref[_ds(r0 // 2, n // 2), :])
        kb = jnp.dot(xb, wk_ref[:, g0 * 128:g1 * 128], preferred_element_type=F32).astype(BF16)
        kf = kb.astype(F32)
        ku = _pk(kb)
        for g in range(g0, g1):
            cols = slice((g - g0) * 128, (g - g0 + 1) * 128)
            k_ref[g, _ds(r0 // 2, n // 2), :] = ku[:, cols]
            for cc in range(n // CK):
                kf_ref[0, g, _ds((r0 // CK + cc) * OFF, OFF), :] = kf[cc * CK + MR:(cc + 1) * CK, cols]
        return _absmax8(kf)

    def qproj(c):
        xb = _upk(xb_ref[_ds(c * (TQ // 2), TQ // 2), :])
        qb = (lax.dot_general(_upk(wqt_ref[...]), xb, nt, preferred_element_type=F32) * QSCALE).astype(BF16)
        qf = qb.astype(F32)
        qu = _pk(qb)
        for g in range(NG):
            qt_ref[g * NQ + c] = qu[g * 64:(g + 1) * 64, :]
            qf_ref[g * NQ + c] = qf[g * 128:(g + 1) * 128, :]
        qa = jnp.abs(qf).reshape(H, 2, 8, TQ)
        return _absmax8(jnp.sum(qa[:, 0] + qa[:, 1], axis=1))

    def vproj(c):
        xi = _upk(xi_ref[_ds(c * (TQ // 2), TQ // 2), :])
        vb = lax.dot_general(_upk(wvt_ref[...]), xi, nt, preferred_element_type=F32).astype(BF16)
        vu = _pk(vb)
        for g in range(NG):
            vt_ref[g, :, _ds(c * TQ, TQ)] = vu[g * 64:(g + 1) * 64, :]
        return _absmax8(vb.astype(F32))

    x_copy(0).start()
    w_copy(0).start()
    w_copy(8).start()
    x_copy(1).start()
    x_copy(2).start()
    w_copy(1).start()
    w_copy(2).start()
    x_copy(3).start()
    x_copy(4).start()
    x_copy(0).wait()
    ln1(0)
    w_copy(0).wait()
    km = kproj(0, XP[1], 0, WS // 128)
    w_copy(8).wait()
    x_copy(1).wait()
    km = jnp.maximum(km, kproj(0, XP[1], WS // 128, NG))
    ln1(1)
    km = jnp.maximum(km, kproj(XP[1], XP[2] - XP[1]))
    x_copy(2).wait()
    w_copy(1).wait()
    wqt_ref[...] = _pk(wq_ref[...].T)
    qm = qproj(0)
    ln1(2)
    km = jnp.maximum(km, kproj(TQ, TQ))
    w_copy(2).wait()
    x_copy(3).wait()
    x_copy(4).wait()
    for i in range(3, 8):
        w_copy(i).start()
    qm = jnp.maximum(qm, qproj(1))
    wvt_ref[...] = _pk(wv_ref[...].T)
    ln1(3)
    vm = vproj(0)
    ln1(4)
    vm = jnp.maximum(vm, vproj(1))

    def proj_body(c, carry):
        km, qm, vm = carry
        return (jnp.maximum(km, kproj(c * TQ, TQ)), jnp.maximum(qm, qproj(c)), jnp.maximum(vm, vproj(c)))

    if P1LOOP:
        km, qm, vm = lax.fori_loop(2, NQ, proj_body, (km, qm, vm))
    else:
        for c in range(2, NQ):
            km, qm, vm = proj_body(c, (km, qm, vm))

    safe = jnp.logical_and(jnp.max(qm) * jnp.max(km) <= SAFE_SCORE, jnp.max(vm) <= SAFE_V)

    def fast_body(it, carry):
        z0 = it >> 8
        z1 = it >> 9
        st = {}
        deps = [None] * (VDEP * NPH)

        blk = [it * NB + b for b in range(NB)]
        grp = [i // NQ for i in blk]

        def qk(b, j, c, n):
            i, g = blk[b], grp[b]
            p_ref = p_refs[n % NPB]

            def emit(r, a, b_, key):
                pa = jnp.exp2(a)
                pb = jnp.exp2(b_)
                p_ref[z0, r * 8:(r + 1) * 8, :] = pltpu.pack_elementwise([pa, pb], packed_dtype=BF16)
                t = pa + pb
                st[key] = t if st[key] is None else st[key] + t

            if c == 0:
                st['l'] = None
                st['l2'] = None

            z = jnp.zeros((8, TQ), U32)
            qm = jnp.concatenate([z] * j + [qt_ref[i, j * 8:(j + 1) * 8, :]] + [z] * (7 - j), axis=0)
            order = list(range(MR // 16))[::-1]
            kc = _upk(jnp.concatenate(
                [k_ref[g, c * CK // 2 + r * 8:c * CK // 2 + (r + 1) * 8, :] for r in order], axis=0))
            s = jnp.dot(kc, _upk(qm), preferred_element_type=F32)
            for ph in range(NPH):
                rr = (ph * (MR // 8) // NPH) * 8
                deps.append(s[rr:rr + 8, DT1 * 128:(DT1 + 1) * 128])
            st['pops', n] = [s[r * 8:(r + 1) * 8, 0:128] for r in range(MR // 8)]
            for q, r in enumerate(order):
                emit(r, s[q * 16:q * 16 + 8], s[q * 16 + 8:q * 16 + 16], 'l')

            accs = [[None] * NL for _ in range(2)]
            for d in range(DH):
                if d % (DH // NPH) == 0:
                    dep = deps[n * NPH + d // (DH // NPH) + PSH]
                    if dep is not None:
                        kf_ref[z0, NG, 0:8, :] = dep
                    if dep is not None or d == 0:
                        kfs = [kf_ref[z1, g, c * OFF + r * 8:c * OFF + (r + 1) * 8, :] for r in range(2)]
                kbs = [jnp.broadcast_to(kf[:, j * DH + d:j * DH + d + 1], (8, 128)) for kf in kfs]
                for t in range(NL):
                    qv = jnp.broadcast_to(qf_ref[i, j * DH + d:j * DH + d + 1, t * 128:(t + 1) * 128], (8, 128))
                    for r in range(2):
                        x = kbs[r] * qv
                        accs[r][t] = x if accs[r][t] is None else accs[r][t] + x
            emit(MR // 16, jnp.concatenate(accs[0], axis=1), jnp.concatenate(accs[1], axis=1), 'l2')
            if c == NC - 1:
                st['inv', b, j] = 1.0 / jnp.sum(st['l'] + st['l2'], axis=0, keepdims=True)

        def pv(b, j, c, n):
            p_ref = p_refs[n % NPB]
            pops = st['pops', min(n + LAG, len(work)) - 1]
            parts = [None] * 8
            for q, r in enumerate(range(7, -1, -1)):
                if q % PGR == 0:
                    p_ref[z0, CK // 2:CK // 2 + 8, 0:128] = _pk(pops[(q * PSP) // 8])
                parts[r] = p_ref[z1, r * 8:(r + 1) * 8, :]
            a = jnp.dot(_upk(vt_ref[grp[b], j * 8:(j + 1) * 8, c * CK:(c + 1) * CK]),
                        _upk(jnp.concatenate(parts, axis=0)), preferred_element_type=F32)
            acc = a if c == 0 else acc_ref[z1] + a
            if c < NC - 1:
                acc_ref[z0] = acc
            else:
                ot_ref[blk[b], j * DH:(j + 1) * DH, :] = (acc * st['inv', b, j]).astype(BF16)

        work = [(b, j, c) for b in range(NB) for j in range(8) for c in range(NC)]
        for n in range(len(work) + LAG):
            if n < len(work):
                qk(*work[n], n)
            if n >= LAG:
                pv(*work[n - LAG], n - LAG)
        return carry

    def slow_body(t, carry):
        i = t // 8
        j = t % 8
        g = i // NQ
        rows = lax.broadcasted_iota(I32, (64, TQ), 0)
        qm = _upk(jnp.where(rows // 8 == j, qt_ref[i], jnp.zeros((64, TQ), U32)))

        def scores(c):
            kc = _upk(k_ref[g, _ds(c * (CK // 2), CK // 2), :])
            return jnp.dot(kc, qm, preferred_element_type=F32)

        def max_body(c, m):
            return jnp.maximum(m, jnp.max(scores(c), axis=0, keepdims=True))

        m = lax.fori_loop(0, NC, max_body, jnp.full((1, TQ), -jnp.inf, F32))

        def acc_body(c, carry):
            acc, l = carry
            p = jnp.exp2(scores(c) - m)
            vc = _upk(vt_ref[g, _ds(j * 8, 8), _ds(c * CK, CK)])
            return (acc + jnp.dot(vc, _upk(_pack_pairs(p)), preferred_element_type=F32),
                    l + jnp.sum(p, axis=0, keepdims=True))

        acc, l = lax.fori_loop(0, NC, acc_body, (jnp.zeros((DH, TQ), F32), jnp.zeros((1, TQ), F32)))
        ot_ref[i, _ds(j * DH, DH), :] = (acc / l).astype(BF16)
        return carry

    @pl.when(safe)
    def _():
        lax.fori_loop(0, 16 // NB, fast_body, 0)

    @pl.when(jnp.logical_not(safe))
    def _():
        lax.fori_loop(0, NG * NQ * 8, slow_body, 0)

    w_copy(3).wait()
    w_copy(4).wait()
    wr16 = jnp.broadcast_to(wr_ref[...].astype(F32).reshape(1, D), (16, D)).astype(BF16)
    nr = S // TR
    top = []

    def otrans(c):
        qb, off = divmod(c * TR, TQ)
        ot = jnp.concatenate([ot_ref[g * NQ + qb, :, off:off + TR] for g in range(NG)], axis=0)
        xb_ref[c * TR // 2:(c + 1) * TR // 2, :] = _pk(ot.T)

    def oproj(c):
        a = jnp.dot(_upk(xb_ref[c * TR // 2:(c + 1) * TR // 2, :]), wo_ref[...], preferred_element_type=F32)
        z_ref[c * TR:(c + 1) * TR, :] = x_ref[c * TR:(c + 1) * TR, :].astype(F32) + a

    def ln2(c):
        h = z_ref[c * TR:(c + 1) * TR, :]
        hn = _layernorm(h)
        zz = h + hn
        hn_ref[c * TR:(c + 1) * TR, :] = hn
        z_ref[c * TR:(c + 1) * TR, :] = zz
        y_ref[c * TR:(c + 1) * TR, :] = zz.astype(BF16)

    def router(c):
        hb = hn_ref[c * TR:(c + 1) * TR, :].astype(BF16)
        r = lax.dot_general(wr16, hb, nt, preferred_element_type=F32)
        rb = pltpu.bitcast(r[0:8].astype(BF16).astype(F32), I32)
        rb = jnp.where(rb < 0, INT_MIN - rb, rb)
        key = rb + (S - 1 - c * TR - lax.broadcasted_iota(I32, (8, TR), 1))
        if c == 0:
            top[:] = [key, jnp.full((8, TR), INT_MIN, I32)]
        else:
            top[:] = [jnp.maximum(top[0], key), jnp.maximum(top[1], jnp.minimum(top[0], key))]

    for c in range(-3, nr + 1):
        if 0 <= c + 3 < nr:
            otrans(c + 3)
        if 0 <= c + 1 < nr:
            oproj(c + 1)
        if 0 <= c - 1 < nr:
            router(c - 1)
        if 0 <= c < nr:
            ln2(c)
            if ((c + 1) * TR) % TQ == 0:
                o_copy(((c + 1) * TR) // TQ - 1).start()

    k1 = jnp.max(top[0])
    k2 = jnp.max(jnp.where(top[0] == k1, top[1], top[0]))
    i1 = jnp.clip((S - 1) - (k1 & 0xFFFF), 0, S - 1)
    i2 = jnp.clip((S - 1) - (k2 & 0xFFFF), 0, S - 1)
    rowi = lax.broadcasted_iota(I32, (16, D), 0)
    xs = jnp.where(rowi == 0, jnp.broadcast_to(hn_ref[pl.ds(i1, 1), :], (16, D)),
                   jnp.broadcast_to(hn_ref[pl.ds(i2, 1), :], (16, D))).astype(BF16)
    ks = jnp.where(rowi == 0, k1, k2) & -65536
    rs = pltpu.bitcast(jnp.where(ks < 0, INT_MIN - ks, ks), F32)
    for i in range(5, 8):
        w_copy(i).wait()
    gg = jnp.dot(xs, wg_ref[...], preferred_element_type=F32)
    uu = jnp.dot(xs, wu_ref[...], preferred_element_type=F32)
    act = (gg * jax.nn.sigmoid(gg) * uu).astype(BF16)
    yy = jnp.dot(act, wd_ref[...], preferred_element_type=F32) * jax.nn.sigmoid(rs)
    y1 = jnp.broadcast_to(yy[0:1], (16, D))
    y2 = jnp.broadcast_to(yy[1:2], (16, D))

    for c in range(NQ):
        o_copy(c).wait()

    def patch(base):
        rr = rowi + base
        blk = z_ref[pl.ds(base, 16), :]
        blk = blk + jnp.where(rr == i1, y1, 0.0) + jnp.where(rr == i2, y2, 0.0)
        y_ref[pl.ds(base, 16), :] = blk.astype(BF16)

    def patch_copy(base, sem):
        return pltpu.make_async_copy(y_ref.at[pl.ds(base, 16)], out_hbm.at[pl.ds(base, 16)], sem)

    b1 = pl.multiple_of((i1 >> 4) << 4, 16)
    b2 = pl.multiple_of((i2 >> 4) << 4, 16)
    patch(b1)
    patch(b2)
    patch_copy(b1, sem_o.at[0]).start()

    @pl.when(b1 != b2)
    def _():
        cp = patch_copy(b2, sem_o.at[1])
        cp.start()
        cp.wait()

    patch_copy(b1, sem_o.at[0]).wait()


@jax.jit
def pallas_sequential_preLN__mha_block__moe_arch_mod__prompt_kernel(
    A_x: jax.Array,
    A_wqkv: jax.Array,
    A_wo: jax.Array,
    B_x: jax.Array,
    B_w_r: jax.Array,
    B_w_gate: jax.Array,
    B_w_up: jax.Array,
    B_w_down: jax.Array,
):
    del B_x
    anyspec = pl.BlockSpec(memory_space=pl.ANY)
    out = pl.pallas_call(
        _kernel,
        out_shape=jax.ShapeDtypeStruct((S, D), BF16),
        in_specs=[anyspec] * 7,
        out_specs=anyspec,
        scratch_shapes=[
            pltpu.VMEM((S, D), BF16),
            pltpu.VMEM((D,), BF16),
            pltpu.VMEM((D, D), BF16),
            pltpu.VMEM((D, D), BF16),
            pltpu.VMEM((D, D), BF16),
            pltpu.VMEM((D, D), BF16),
            pltpu.VMEM((D, FF), BF16),
            pltpu.VMEM((D, FF), BF16),
            pltpu.VMEM((FF, D), BF16),
            pltpu.VMEM((S // 2, D), U32),
            pltpu.VMEM((S // 2, D), U32),
            pltpu.VMEM((D // 2, D), U32),
            pltpu.VMEM((D // 2, D), U32),
            pltpu.VMEM((NG, S // 2, 128), U32),
            pltpu.VMEM((1, NG + 1, NC * OFF, 128), F32),
            pltpu.VMEM((NG * NQ, 64, TQ), U32),
            pltpu.VMEM((NG * NQ, 128, TQ), F32),
            pltpu.VMEM((NG, 64, S), U32),
            pltpu.VMEM((NG * NQ, 128, TQ), BF16),
            pltpu.VMEM((1, DH, TQ), F32),
            pltpu.VMEM((S, D), F32),
            pltpu.VMEM((S, D), F32),
            pltpu.VMEM((S, D), BF16),
        ] + [pltpu.VMEM((1, CK // 2 + 8, TQ), U32)] * NPB + [
            pltpu.SemaphoreType.DMA((len(XP) - 1,)),
            pltpu.SemaphoreType.DMA((9,)),
            pltpu.SemaphoreType.DMA((NQ,)),
        ],
        compiler_params=pltpu.CompilerParams(vmem_limit_bytes=100 * 1024 * 1024),
    )(A_x.reshape(S, D), A_wqkv, A_wo, B_w_r, B_w_gate, B_w_up, B_w_down)
    return out.reshape(1, S, D)
```

```python
import math

import jax
import jax.numpy as jnp
from jax import lax
from jax.experimental import pallas as pl
from jax.experimental.pallas import tpu as pltpu

F32 = jnp.float32
BF16 = jnp.bfloat16
U32 = jnp.uint32
I32 = jnp.int32

S = 2048
D = 512
H = 32
DH = 16
FF = 1792
TQ = 512
CK = 128
NQ = S // TQ
NC = S // CK
NL = TQ // 128
NG = D // 128
OFF = 16
TR = 128
WS = 256
XP = (0, 384, 640, 1024, 1536, 2048)
EPS = 1e-5
EPS_BF16 = 1.0013580322265625e-05
QSCALE = (DH ** -0.5) * math.log2(math.e)
INT_MIN = -2 ** 31
SAFE_SCORE = 96.0
SAFE_WV = 100.0
PLAN = ("EESSSVSS", "EESSVSSS", "EESSVSSS", "ESVSSSSS", "EEVSSSSS", "EEVSSSSS", "EEVSSSSS", "EEVSSSVS",
        "EESSSVSS", "EESSVSSS", "EESVSSSS", "EEVSSSSS", "EEVSSSSS", "EEVSSSSS", "EEVSSSSS", "EEVSSSVS")
V_DONE = 190
V_LAT = 130


def _rows(c, kind):
    return [7 - q for q, v in enumerate(PLAN[c]) if v == kind]


def _stream(c, first=False):
    own = [(c, r) for r in (_rows(c, "E") if first else []) + _rows(c, "S")]
    return own + ([(c + 1, r) for r in _rows(c + 1, "E")] if c < NC - 1 else [])


UNITS = [(c, r) for c in range(NC) for r in _rows(c, "V")]
NU = len(UNITS)
START = [sum(16 * len(_stream(q)) + 16 for q in range(c)) for c in range(NC + 1)]
NE0 = len(_rows(0, "E"))
START[NC] += 16 * NE0
GATE = [[V_DONE + u * START[NC] / NU - V_LAT - (DH - 2 - d) * START[NC] / NU / DH for d in range(DH)]
        for u in range(NU)]


def _pk(x):
    return pltpu.bitcast(x, U32)


def _upk(x):
    return pltpu.bitcast(x, BF16)


def _ds(start, size):
    if isinstance(start, int):
        return pl.ds(start, size)
    return pl.ds(pl.multiple_of(start, size), size)


def _layernorm(x):
    m = jnp.mean(x, axis=-1, keepdims=True)
    xc = x - m
    v = jnp.mean(xc * xc, axis=-1, keepdims=True)
    return xc * lax.rsqrt(v + EPS)


def _rb(x):
    return x.astype(BF16).astype(F32)


def _layernorm_bf16(x):
    m = jnp.mean(x, axis=-1, keepdims=True)
    xc = x - m
    v = jnp.mean(xc * xc, axis=-1, keepdims=True)
    d = _rb(jnp.sqrt(_rb(_rb(v) + EPS_BF16)))
    return _rb(x - _rb(m)) / d


def _absmax8(x):
    r, c = x.shape
    a = jnp.abs(x).reshape(r // 8, 8, c).max(axis=0)
    out = a[:, 0:128]
    for t in range(1, c // 128):
        out = jnp.maximum(out, a[:, t * 128:(t + 1) * 128])
    return out


def _kernel(x_hbm, wqkv_hbm, wo_hbm, wr_hbm, wg_hbm, wu_hbm, wd_hbm, out_hbm,
            x_ref, wr_ref, wq_ref, wka_ref, wkb_ref, wv_ref, wo_ref, wg_ref, wu_ref, wd_ref,
            xb_ref, wqt_ref, wvt_ref, k_ref, kf_ref, qt_ref, qf_ref, vt_ref, ot_ref,
            acc_ref, l_ref, hn_ref, z_ref, y_ref, p0, sem_x, sem_w, sem_o):
    nt = (((1,), (1,)), ((), ()))

    def x_copy(c):
        rows = pl.ds(XP[c], XP[c + 1] - XP[c])
        return pltpu.make_async_copy(x_hbm.at[rows], x_ref.at[rows], sem_x.at[c])

    def w_copy(i):
        src, dst = ((wqkv_hbm.at[:, pl.ds(D, WS)], wka_ref),
                    (wqkv_hbm.at[:, pl.ds(0, D)], wq_ref),
                    (wqkv_hbm.at[:, pl.ds(2 * D, D)], wv_ref), (wo_hbm, wo_ref), (wr_hbm, wr_ref),
                    (wg_hbm, wg_ref), (wu_hbm, wu_ref), (wd_hbm, wd_ref),
                    (wqkv_hbm.at[:, pl.ds(D + WS, D - WS)], wkb_ref))[i]
        return pltpu.make_async_copy(src, dst, sem_w.at[i])

    def o_copy(c):
        rows = pl.ds(c * TQ, TQ)
        return pltpu.make_async_copy(y_ref.at[rows], out_hbm.at[rows], sem_o.at[c])

    def ln1(c):
        r0, r1 = XP[c], XP[c + 1]
        xn = _layernorm(x_ref[r0:r1, :].astype(F32))
        xb_ref[r0 // 2:r1 // 2, :] = _pk(xn.astype(BF16))

    def kproj(r0, n, g0=0, g1=NG, store_kf=True):
        xb = _upk(xb_ref[_ds(r0 // 2, n // 2), :])
        wk = [r[...] for r, lo in ((wka_ref, 0), (wkb_ref, WS // 128)) if g0 <= lo < g1]
        kb = jnp.dot(xb, jnp.concatenate(wk, axis=1), preferred_element_type=F32).astype(BF16)
        kf = kb.astype(F32)
        ku = _pk(kb)
        for g in range(g0, g1):
            cols = slice((g - g0) * 128, (g - g0 + 1) * 128)
            k_ref[g, _ds(r0 // 2, n // 2), :] = ku[:, cols]
            for cc in range(n // CK):
                for u, (uc, ur) in enumerate(UNITS):
                    if store_kf and uc == r0 // CK + cc:
                        row = cc * CK + ur * OFF
                        kf_ref[0, g, u * DH * OFF:u * DH * OFF + OFF, :] = kf[row:row + OFF, cols]
        return _absmax8(kf)

    def kroll(c0, c1):
        for g in range(NG):
            for u in [u for u, (uc, _) in enumerate(UNITS) if c0 <= uc < c1]:
                kv = kf_ref[0, g, u * DH * OFF:u * DH * OFF + OFF, :]
                for d in range(1, DH):
                    kf_ref[0, g, (u * DH + d) * OFF:(u * DH + d + 1) * OFF, :] = pltpu.roll(kv, 128 - d, axis=1)

    def qproj(c):
        xb = _upk(xb_ref[_ds(c * (TQ // 2), TQ // 2), :])
        qb = (lax.dot_general(_upk(wqt_ref[...]), xb, nt, preferred_element_type=F32) * QSCALE).astype(BF16)
        qf = qb.astype(F32)
        qu = _pk(qb)
        for g in range(NG):
            qt_ref[g * NQ + c] = qu[g * 64:(g + 1) * 64, :]
            qf_ref[g * NQ + c] = qf[g * 128:(g + 1) * 128, :]
        qa = jnp.abs(qf).reshape(H, 2, 8, TQ)
        return _absmax8(jnp.sum(qa[:, 0] + qa[:, 1], axis=1))

    def vproj(c):
        xi = _upk(xb_ref[_ds(c * (TQ // 2), TQ // 2), :])
        vb = lax.dot_general(_upk(wvt_ref[...]), xi, nt, preferred_element_type=F32).astype(BF16)
        vu = _pk(vb)
        for g in range(NG):
            vt_ref[g, :, _ds(c * TQ, TQ)] = vu[g * 64:(g + 1) * 64, :]

    x_copy(0).start()
    w_copy(0).start()
    w_copy(8).start()
    x_copy(1).start()
    x_copy(2).start()
    w_copy(1).start()
    w_copy(2).start()
    x_copy(3).start()
    x_copy(4).start()
    p0[...] = jnp.zeros(p0.shape, BF16)
    acc_ref[...] = jnp.zeros(acc_ref.shape, F32)
    l_ref[...] = jnp.ones(l_ref.shape, F32)
    ot_ref[NG * NQ - 1, 7 * DH:8 * DH, :] = jnp.zeros((DH, TQ), BF16)
    x_copy(0).wait()
    ln1(0)
    w_copy(0).wait()
    km = kproj(0, XP[1], 0, WS // 128)
    w_copy(8).wait()
    x_copy(1).wait()
    km = jnp.maximum(km, kproj(0, XP[1], WS // 128, NG))
    ln1(1)
    km = jnp.maximum(km, kproj(XP[1], XP[2] - XP[1]))
    x_copy(2).wait()
    w_copy(1).wait()
    wqt_ref[...] = _pk(wq_ref[...].T)
    qm = qproj(0)
    ln1(2)
    km = jnp.maximum(km, kproj(XP[2], XP[3] - XP[2]))
    w_copy(2).wait()
    x_copy(3).wait()
    x_copy(4).wait()
    for i in range(3, 8):
        w_copy(i).start()
    qm = jnp.maximum(qm, qproj(1))
    wvt_ref[...] = _pk(wv_ref[...].T)
    ln1(3)
    vm = _absmax8(wv_ref[...].astype(F32))
    vproj(0)
    ln1(4)
    vproj(1)
    kroll(0, 8)
    for c in range(2, NQ):
        km = jnp.maximum(km, kproj(c * TQ, TQ))
        qm = jnp.maximum(qm, qproj(c))
        kroll(4 * c, 4 * c + 4)
        vproj(c)

    safe = jnp.logical_and(jnp.max(qm) * jnp.max(km) <= SAFE_SCORE, jnp.max(vm) <= SAFE_WV)

    def pv_chunk(z0, z1, i, g, j, c, p, inv):
        a = jnp.dot(_upk(vt_ref[g, j * 8:(j + 1) * 8, c * CK:(c + 1) * CK]), p, preferred_element_type=F32)
        acc = a if c == 0 else acc_ref[z1] + a
        if c < NC - 1:
            acc_ref[z0] = acc
        else:
            ot_ref[i, j * DH:(j + 1) * DH, :] = (acc * inv).astype(BF16)

    def pv_carried(z0, z1, i, g):
        inv = 1.0 / jnp.sum(l_ref[...], axis=0, keepdims=True)
        pv_chunk(z0, z1, i, g, 7, NC - 1, p0[...], inv)

    def fast_body(it, carry):
        z0 = it >> 8
        z1 = it >> 9
        g = it >> 2
        st = {}
        pops = []
        nw = 8 * NC

        def emit(n, r, x):
            j = n // NC
            p = jnp.exp2(x)
            if n == nw - 1:
                p0[r * 16:(r + 1) * 16, :] = p.astype(BF16)
            else:
                st['p', n, r] = p
            t = p[0:8] + p[8:16]
            st['l', j] = st['l', j] + t if ('l', j) in st else t

        def scores(j, groups, t):
            z = jnp.zeros((8, TQ), U32)
            qm = jnp.concatenate([z] * j + [qt_ref[it, j * 8:(j + 1) * 8, :]] + [z] * (7 - j), axis=0)
            kc = _upk(jnp.concatenate(
                [k_ref[g, m * 64 + r * 8:m * 64 + (r + 1) * 8, :] for m, r in groups], axis=0))
            s = jnp.dot(kc, _upk(qm), preferred_element_type=F32)
            pops.extend((t + 125 + 8 * q, s, q) for q in range(2 * len(groups)))
            return s

        def qk(n):
            j, c = divmod(n, NC)
            groups = _stream(c, n == 0)
            t0 = j * START[NC]
            s = scores(j, groups, t0 + START[c] - (16 * NE0 if n == 0 else 0))
            if c == NC - 1 and j < 7:
                nxt = [(0, r) for r in _rows(0, "E")]
                s2 = scores(j + 1, nxt, t0 + START[c] + 16 * len(groups))

            for u, (uc, ur) in enumerate(UNITS):
                if uc != c:
                    continue
                acc = None
                for d in range(DH):
                    if d % 2 == 0:
                        seen = [p for p in pops if p[0] <= t0 + GATE[u][d]]
                        if seen:
                            _, src, q = seen[-1]
                            kf_ref[z0, NG, 0:8, :] = src[q * 8:q * 8 + 8, 0:128]
                    if u == 0:
                        st['qv', d] = jnp.concatenate([jnp.broadcast_to(
                            qf_ref[it, j * DH + d:j * DH + d + 1, t * 128:(t + 1) * 128], (OFF, 128))
                            for t in range(NL)], axis=1)
                    kf = kf_ref[z1, g, (u * DH + d) * OFF:(u * DH + d + 1) * OFF, :]
                    x = kf[:, j * DH:j * DH + 1] * st['qv', d]
                    acc = x if acc is None else acc + x
                emit(n, ur, acc)
            for q, (m, r) in enumerate(groups):
                emit(j * NC + m, r, s[q * 16:(q + 1) * 16])
            if c == NC - 1 and j < 7:
                for q, (m, r) in enumerate(nxt):
                    emit(n + 1, r, s2[q * 16:(q + 1) * 16])

        def pv(n):
            j, c = divmod(n, NC)
            p = jnp.concatenate([st.pop(('p', n, r)) for r in range(8)], axis=0).astype(BF16)
            inv = 1.0 / jnp.sum(st['l', j], axis=0, keepdims=True) if c == NC - 1 else None
            pv_chunk(z0, z1, it, g, j, c, p, inv)

        for n in range(nw):
            qk(n)
            if n > 0:
                pv(n - 1)
            else:
                pv_carried(z0, z1, jnp.where(it == 0, NG * NQ, it - 1), jnp.maximum(it - 1, 0) >> 2)
        l_ref[...] = st['l', 7]
        return carry

    def slow_body(t, carry):
        i = t // 8
        j = t % 8
        g = i // NQ
        rows = lax.broadcasted_iota(I32, (64, TQ), 0)
        qm = _upk(jnp.where(rows // 8 == j, qt_ref[i], jnp.zeros((64, TQ), U32)))

        def scores(c):
            kc = _upk(k_ref[g, _ds(c * (CK // 2), CK // 2), :])
            return _rb(jnp.dot(kc, qm, preferred_element_type=F32)) * QSCALE

        def max_body(c, m):
            return jnp.maximum(m, jnp.max(scores(c), axis=0, keepdims=True))

        m = lax.fori_loop(0, NC, max_body, jnp.full((1, TQ), -jnp.inf, F32))

        def acc_body(c, carry):
            acc, l = carry
            p = jnp.exp2(scores(c) - m)
            vc = _upk(vt_ref[g, _ds(j * 8, 8), _ds(c * CK, CK)])
            return (acc + jnp.dot(vc, p.astype(BF16), preferred_element_type=F32),
                    l + jnp.sum(p, axis=0, keepdims=True))

        acc, l = lax.fori_loop(0, NC, acc_body, (jnp.zeros((DH, TQ), F32), jnp.zeros((1, TQ), F32)))
        ot_ref[i, _ds(j * DH, DH), :] = (acc / l).astype(BF16)
        return carry

    def reproject(c, carry):
        xn = _layernorm_bf16(x_ref[_ds(c * TQ, TQ), :].astype(F32))
        xb_ref[_ds(c * (TQ // 2), TQ // 2), :] = _pk(xn.astype(BF16))
        kproj(c * TQ, TQ, store_kf=False)
        vproj(c)
        xb = _upk(xb_ref[_ds(c * (TQ // 2), TQ // 2), :])
        qu = _pk(lax.dot_general(_upk(wqt_ref[...]), xb, nt, preferred_element_type=F32).astype(BF16))
        for g in range(NG):
            qt_ref[g * NQ + c] = qu[g * 64:(g + 1) * 64, :]
        return carry

    def fast_path():
        lax.fori_loop(0, NG * NQ, fast_body, 0)

    def slow_path():
        lax.fori_loop(0, NQ, reproject, 0)
        lax.fori_loop(0, NG * NQ * 8, slow_body, 0)

    lax.cond(safe, fast_path, slow_path)

    w_copy(3).wait()
    w_copy(4).wait()
    wr16 = jnp.broadcast_to(wr_ref[...].astype(F32).reshape(1, D), (16, D)).astype(BF16)
    nr = S // TR
    top = []

    def otrans(c):
        qb, off = divmod(c * TR, TQ)
        ot = jnp.concatenate([ot_ref[g * NQ + qb, :, off:off + TR] for g in range(NG)], axis=0)
        xb_ref[c * TR // 2:(c + 1) * TR // 2, :] = _pk(ot.T)

    def oproj(c):
        a = jnp.dot(_upk(xb_ref[c * TR // 2:(c + 1) * TR // 2, :]), wo_ref[...], preferred_element_type=F32)
        z_ref[c * TR:(c + 1) * TR, :] = x_ref[c * TR:(c + 1) * TR, :].astype(F32) + a

    def ln2(c):
        h = z_ref[c * TR:(c + 1) * TR, :]
        hn = _layernorm(h)
        zz = h + hn
        hn_ref[c * TR:(c + 1) * TR, :] = hn
        z_ref[c * TR:(c + 1) * TR, :] = zz
        y_ref[c * TR:(c + 1) * TR, :] = zz.astype(BF16)

    def router(c):
        hb = hn_ref[c * TR:(c + 1) * TR, :].astype(BF16)
        r = lax.dot_general(wr16, hb, nt, preferred_element_type=F32)
        rb = pltpu.bitcast(r[0:8].astype(BF16).astype(F32), I32)
        rb = jnp.where(rb < 0, INT_MIN - rb, rb)
        key = rb + (S - 1 - c * TR - lax.broadcasted_iota(I32, (8, TR), 1))
        if c == 0:
            top[:] = [key, jnp.full((8, TR), INT_MIN, I32)]
        else:
            top[:] = [jnp.maximum(top[0], key), jnp.maximum(top[1], jnp.minimum(top[0], key))]

    for c in range(-3, nr + 1):
        if 0 <= c + 3 < nr:
            otrans(c + 3)
        if c == -1:
            pv_carried(0, 0, jnp.where(safe, NG * NQ - 1, NG * NQ), NG - 1)
        if 0 <= c + 1 < nr:
            oproj(c + 1)
        if 0 <= c - 1 < nr:
            router(c - 1)
        if 0 <= c < nr:
            ln2(c)
            if ((c + 1) * TR) % TQ == 0:
                o_copy(((c + 1) * TR) // TQ - 1).start()

    k1 = jnp.max(top[0])
    k2 = jnp.max(jnp.where(top[0] == k1, top[1], top[0]))
    i1 = jnp.clip((S - 1) - (k1 & 0xFFFF), 0, S - 1)
    i2 = jnp.clip((S - 1) - (k2 & 0xFFFF), 0, S - 1)
    rowi = lax.broadcasted_iota(I32, (16, D), 0)
    xs = jnp.where(rowi == 0, jnp.broadcast_to(hn_ref[pl.ds(i1, 1), :], (16, D)),
                   jnp.broadcast_to(hn_ref[pl.ds(i2, 1), :], (16, D))).astype(BF16)
    ks = jnp.where(rowi == 0, k1, k2) & -65536
    rs = pltpu.bitcast(jnp.where(ks < 0, INT_MIN - ks, ks), F32)
    for i in range(5, 8):
        w_copy(i).wait()
    gg = jnp.dot(xs, wg_ref[...], preferred_element_type=F32)
    uu = jnp.dot(xs, wu_ref[...], preferred_element_type=F32)
    act = (gg * jax.nn.sigmoid(gg) * uu).astype(BF16)
    yy = jnp.dot(act, wd_ref[...], preferred_element_type=F32) * jax.nn.sigmoid(rs)
    y1 = jnp.broadcast_to(yy[0:1], (16, D))
    y2 = jnp.broadcast_to(yy[1:2], (16, D))

    for c in range(NQ):
        o_copy(c).wait()

    def patch(base):
        rr = rowi + base
        blk = z_ref[pl.ds(base, 16), :]
        blk = blk + jnp.where(rr == i1, y1, 0.0) + jnp.where(rr == i2, y2, 0.0)
        y_ref[pl.ds(base, 16), :] = blk.astype(BF16)

    def patch_copy(base, sem):
        return pltpu.make_async_copy(y_ref.at[pl.ds(base, 16)], out_hbm.at[pl.ds(base, 16)], sem)

    b1 = pl.multiple_of(jnp.clip(i1 >> 4, 0, S // 16 - 1) * 16, 16)
    b2 = pl.multiple_of(jnp.clip(i2 >> 4, 0, S // 16 - 1) * 16, 16)
    patch(b1)
    patch(b2)
    for base in (b1, b2):
        cp = patch_copy(base, sem_o.at[0])
        cp.start()
        cp.wait()


@jax.jit
def pallas_sequential_preLN__mha_block__moe_arch_mod__prompt_kernel(
    A_x: jax.Array,
    A_wqkv: jax.Array,
    A_wo: jax.Array,
    B_x: jax.Array,
    B_w_r: jax.Array,
    B_w_gate: jax.Array,
    B_w_up: jax.Array,
    B_w_down: jax.Array,
):
    del B_x
    anyspec = pl.BlockSpec(memory_space=pl.ANY)
    out = pl.pallas_call(
        _kernel,
        out_shape=jax.ShapeDtypeStruct((S, D), BF16),
        in_specs=[anyspec] * 7,
        out_specs=anyspec,
        scratch_shapes=[
            pltpu.VMEM((S, D), BF16),
            pltpu.VMEM((D,), BF16),
            pltpu.VMEM((D, D), BF16),
            pltpu.VMEM((D, WS), BF16),
            pltpu.VMEM((D, D - WS), BF16),
            pltpu.VMEM((D, D), BF16),
            pltpu.VMEM((D, D), BF16),
            pltpu.VMEM((D, FF), BF16),
            pltpu.VMEM((D, FF), BF16),
            pltpu.VMEM((FF, D), BF16),
            pltpu.VMEM((S // 2, D), U32),
            pltpu.VMEM((D // 2, D), U32),
            pltpu.VMEM((D // 2, D), U32),
            pltpu.VMEM((NG, S // 2, 128), U32),
            pltpu.VMEM((1, NG + 1, NU * DH * OFF, 128), F32),
            pltpu.VMEM((NG * NQ, 64, TQ), U32),
            pltpu.VMEM((NG * NQ, 128, TQ), F32),
            pltpu.VMEM((NG, 64, S), U32),
            pltpu.VMEM((NG * NQ + 1, 128, TQ), BF16),
            pltpu.VMEM((1, DH, TQ), F32),
            pltpu.VMEM((8, TQ), F32),
            pltpu.VMEM((S, D), F32),
            pltpu.VMEM((S, D), F32),
            pltpu.VMEM((S, D), BF16),
            pltpu.VMEM((CK, TQ), BF16),
            pltpu.SemaphoreType.DMA((len(XP) - 1,)),
            pltpu.SemaphoreType.DMA((9,)),
            pltpu.SemaphoreType.DMA((NQ,)),
        ],
        compiler_params=pltpu.CompilerParams(vmem_limit_bytes=100 * 1024 * 1024),
    )(A_x.reshape(S, D), A_wqkv, A_wo, B_w_r, B_w_gate, B_w_up, B_w_down)
    return out.reshape(1, S, D)
```
